```python
import jax
import jax.numpy as jnp

def _softmax(x, axis=-1):
    return jax.nn.softmax(x, axis=axis)

def _gelu(x):
    return jax.nn.gelu(x, approximate=True)

def _silu(x):
    return jax.nn.silu(x)

def _sigmoid(x):
    return jax.nn.sigmoid(x)

def _layernorm(x, axis=-1, eps=1e-05):
    m = jnp.mean(x, axis=axis, keepdims=True)
    v = jnp.var(x, axis=axis, keepdims=True)
    return (x - m) / jnp.sqrt(v + eps)

def _scatter_add(tgt, idx, src, axis=0):
    return tgt.at[idx].add(src)

def _segment_sum(src, seg, n):
    return jax.ops.segment_sum(src, seg, n)

class _Rng:

    def __init__(self, key):
        self._k = key

    def _next(self):
        self._k, sub = jax.random.split(self._k)
        return sub

    def normal(self, shape):
        return jax.random.normal(self._next(), shape, dtype=jnp.bfloat16)

    def randint(self, lo, hi, shape):
        return jax.random.randint(self._next(), shape, lo, hi, dtype=jnp.int32)

    def uniform(self, shape, lo=0.0, hi=1.0):
        return jax.random.uniform(self._next(), shape, jnp.bfloat16, lo, hi)

    def permutation(self, n):
        return jax.random.permutation(self._next(), n)
kernel_name = 'adaLN_cond__sliding_block_cached__dense_activation_mish__decode'

def setup_inputs():
    _rng = _Rng(jax.random.key(int.from_bytes(__import__("os").urandom(4), "little")))
    _w = lambda a: (lambda t: t.astype(jnp.bfloat16) if jnp.issubdtype(t.dtype, jnp.floating) else t)(jnp.asarray(a))

    def _A_setup():
        B, Sq, D = (1, 1, 640)
        Hq, Hkv, Sk, Dh = (32, 32, 32768, 192)
        assert Hq % Hkv == 0, (Hq, Hkv)
        return {'x': _w((lambda *s: _rng.normal(s) * 0.05)(B, Sq, D)), 'k_cache': _w((lambda *s: _rng.normal(s) * 0.05)(B, Hkv, Sk, Dh)), 'v_cache': _w((lambda *s: _rng.normal(s) * 0.05)(B, Hkv, Sk, Dh)), 'wq': _w((lambda *s: _rng.normal(s) * 0.05)(D, Hq * Dh) * D ** (-0.5)), 'wo': _w((lambda *s: _rng.normal(s) * 0.05)(Hq * Dh, D) * (Hq * Dh) ** (-0.5))}
    _A_in = _A_setup()

    def _B_setup():
        B, S, D, F = (1, 1, 640, 1536)
        return {'x': _w((lambda *s: _rng.normal(s) * 0.05)(B, S, D)), 'w1': _w((lambda *s: _rng.normal(s) * 0.05)(D, F) * D ** (-0.5)), 'b1': _w((lambda *s: _rng.normal(s) * 0.05)(F)), 'w2': _w((lambda *s: _rng.normal(s) * 0.05)(F, D) * F ** (-0.5))}
    _B_in = _B_setup()
    return {'A_x': _A_in['x'], 'A_k_cache': _A_in['k_cache'], 'A_v_cache': _A_in['v_cache'], 'A_wq': _A_in['wq'], 'A_wo': _A_in['wo'], 'B_x': _B_in['x'], 'B_w1': _B_in['w1'], 'B_b1': _B_in['b1'], 'B_w2': _B_in['w2'], 'c': _w((lambda *s: _rng.normal(s) * 0.05)(1, 640)), 'w_mod': _w((lambda *s: _rng.normal(s) * 0.05)(640, 6 * 640) * 640 ** (-0.5))}

def reference(A_x, A_k_cache, A_v_cache, A_wq, A_wo, B_x, B_w1, B_b1, B_w2, c, w_mod):

    def _A_ref(x, k_cache, v_cache, wq, wo):
        B, Sq, D = x.shape
        Hq, Dh = (32, 192)
        Hkv, Sk = (k_cache.shape[1], k_cache.shape[2])
        W = min(4096, max(256, Sk // 4))
        rep = Hq // Hkv
        q = (lambda x, *d: x.transpose(*d))((x @ wq).reshape(B, Sq, Hq, Dh), 0, 2, 1, 3)
        k = jnp.repeat(k_cache[:, :, Sk - W:, :], rep, axis=1)
        v = jnp.repeat(v_cache[:, :, Sk - W:, :], rep, axis=1)
        scores = jnp.einsum('bhqd,bhkd->bhqk', q, k) * Dh ** (-0.5)
        p = _softmax(scores, axis=-1)
        o = jnp.einsum('bhqk,bhkd->bhqd', p, v)
        return (lambda x, *d: x.transpose(*d))(o, 0, 2, 1, 3).reshape(B, Sq, Hq * Dh) @ wo

    def _B_ref(x, w1, b1, w2):
        h = jnp.einsum('bsd,df->bsf', x, w1) + b1
        sp = jnp.log1p(jnp.exp(-jnp.abs(h))) + jnp.where(h > 0, h, jnp.zeros_like(h))
        act = h * jnp.tanh(sp)
        return jnp.einsum('bsf,fd->bsd', act, w2)
    x = A_x
    mod = (_silu(c) @ w_mod).reshape(c.shape[0], 6, 1, -1)
    sa, ca, ga, sb, cb, gb = (mod[:, 0].copy(), mod[:, 1].copy(), mod[:, 2].copy(), mod[:, 3].copy(), mod[:, 4].copy(), mod[:, 5].copy())
    h = _layernorm(x, axis=-1) * (1 + ca) + sa
    x = x + ga * _A_ref(h, A_k_cache, A_v_cache, A_wq, A_wo)
    h = _layernorm(x, axis=-1) * (1 + cb) + sb
    x = x + gb * _B_ref(h, B_w1, B_b1, B_w2)
    return x
```

```python
import functools

import jax
import jax.numpy as jnp
from jax import lax
import jax.experimental.pallas as pl
import jax.experimental.pallas.tpu as pltpu

D = 640
H = 32
DH = 192
F = 1536
PAIR = 2 * DH
NPAIR = H // 2
LANE = 128
ND = D // LANE
NF = F // LANE
F32 = jnp.float32
BF16 = jnp.bfloat16

SLAB = 2048
RUN = 32
KV_ROWS, KV_COLS = 32, 512
HALF = 24
W_LEAD = 24
LEAD = 27
NSLOT = 3
V_GROUPS = (3, 2, 2, 1)
W2_MXU = (28, 20)
W2_VPU = (4, 4, 2, 1, 1)
W2_BOTH = 36


def _tile_major(w):
    r, c = w.shape
    return w.reshape(r // 8, 8, c // LANE, LANE).transpose(0, 2, 1, 3).reshape(-1, LANE)


def _iota(shape, dim):
    return lax.broadcasted_iota(jnp.int32, shape, dim)


def _row(v, i, rows=8):
    return jnp.broadcast_to(v[i:i + 1], (rows, v.shape[1]))


def _stack(v):
    out = jnp.zeros((8, LANE), F32)
    for j in range(v.shape[1] // LANE):
        out = jnp.where(_iota((8, LANE), 0) == j, _row(v[:, j * LANE:(j + 1) * LANE], 0), out)
    return out


def _tile_coords(block, width, shape):
    i = _iota(shape, 1) >> 3
    r0, c0 = divmod(16 * block, width)
    r, c = jnp.full(shape, r0, jnp.int32), i + c0
    for k in range(width - c0, 16, width):
        r = jnp.where(i >= k, r + 1, r)
        c = jnp.where(i >= k, c - width, c)
    return r, c


def _selector(width):
    shape = (LANE, LANE)
    source = lambda m: _tile_coords(m, width, shape)[0] * 8 + (_iota(shape, 1) & 7)
    return jnp.concatenate([jnp.where(source(m) == _iota(shape, 0), 1.0, 0.0).astype(BF16)
                            for m in range(width)], axis=1)


def _layernorm(x, eps=1e-5):
    total = lambda a: jnp.sum(jnp.sum(a, axis=1, keepdims=True), axis=0, keepdims=True)
    d = jnp.where(_iota(x.shape, 0) < ND, x - total(x) / D, 0.0)
    return d / jnp.sqrt(total(d * d) / D + eps)


def _mish(u):
    softplus = jnp.log1p(jnp.exp(-jnp.abs(u))) + jnp.where(u > 0, u, 0.0)
    return u * jnp.tanh(softplus)


def _dot(a, b):
    return jnp.dot(a, b, preferred_element_type=F32)


def _loop(lo, hi, body):
    lax.fori_loop(lo, hi, lambda i, carry: (body(i), carry)[1], 0)


def _aligned(i, n):
    return i if isinstance(i, int) else pl.multiple_of(i, n)


def _starts(sizes):
    return [sum(sizes[:i]) for i in range(len(sizes) + 1)]


def _wait(buf, sem):
    pltpu.make_async_copy(buf, buf, sem).wait()


def _kernel(x_hbm, k_hbm, v_hbm, wq_hbm, wo_hbm, w1_hbm, b1_hbm, w2_hbm, c_hbm, wm_hbm, o_ref,
            x_v, c_v, b1_v, wm_v, wq_v, wo_v, w1_v, w2_v, kv_v,
            q_s, e_s, den_s, sel_d, sel_f, col_d, col_f, g_s, acc_s, y_s, a_s,
            sem_w, sem_kv, sem_v, sem_w2, fence):
    window = kv_v.shape[-1]
    col0 = k_hbm.shape[1] - window
    copy = lambda src, dst, sem: functools.partial(pltpu.make_async_copy, src, dst, sem)

    def start(first, second):
        for i in range(max(len(first), len(second))):
            for queue, copies in enumerate((first, second)):
                if i < len(copies):
                    pl.semaphore_signal(fence, 1)
                    pl.semaphore_wait(fence, 1)
                    copies[i]().start(priority=queue)

    def runs(weight, slab, nslab, run):
        src, dst, sem = weight
        n = src.shape[0] // SLAB
        whole = lambda ref: ref if ref.shape[0] == n * SLAB else ref.at[pl.ds(0, n * SLAB)]
        at = (pl.ds(slab, nslab), pl.ds(_aligned(run * RUN, RUN), RUN))
        return copy(whole(src).reshape(n, SLAB, LANE).at[at], whole(dst).reshape(n, SLAB, LANE).at[at], sem)

    def block(weight, b):
        src, dst, sem = weight
        return copy(src.at[pl.ds(b * LANE, LANE)], dst.at[pl.ds(b * LANE, LANE)], sem)

    def slot_of(src, p):
        return (p + (NPAIR if src is v_hbm else 0)) % NSLOT

    def half_head(src, p, which, half, sem_of=None):
        slot = slot_of(src, p)
        return [copy(src.at[pl.ds(_aligned(p * PAIR + r, KV_ROWS), KV_ROWS), pl.ds(col0 + c, KV_COLS)],
                     kv_v.at[slot, pl.ds(r, KV_ROWS), pl.ds(c, KV_COLS)],
                     sem_of(c) if sem_of else sem_kv.at[slot])
                for c in range(0, window, KV_COLS)
                for r in range(which * DH + half * DH // 2, which * DH + (half + 1) * DH // 2, KV_ROWS)]

    def start_head(src, p, which, later=None):
        if later is None:
            later = half_head(src, p + which, 1 - which, 1) + half_head(src, p + 1, which, 1)
        start(half_head(src, p, which, 0), later[LEAD - HALF:LEAD])

    def start_pair(src, p):
        start_head(src, p, 0)
        start_head(src, p, 1)

    wm, w1 = (wm_hbm, wm_v, sem_w.at[0]), (w1_hbm, w1_v, sem_w.at[1])
    wq, wo = (wq_hbm, wq_v.reshape(wq_hbm.shape), sem_w.at[2]), (wo_hbm, wo_v, sem_w.at[3])
    small = [copy(s, d, sem_w.at[4 + i]) for i, (s, d) in enumerate(((c_hbm, c_v), (x_hbm, x_v), (b1_hbm, b1_v)))]
    first_a = lambda r: [runs(wm, s, 3, r) for s in (0, 3, 6)]
    first_b = lambda r: [runs(wq, 12, 3, r), runs(wo, 12, 3, r), runs(w1, 0, 3, r)]
    second_a = lambda r: [runs(wq, s, 4, r) for s in (0, 4, 8)]
    second_b = lambda r: [runs(wo, s, 4, r) for s in (0, 4, 8)]
    over = lambda copies, lo, hi: [cp for r in range(lo, hi) for cp in copies(r)]
    nrun, (lead, skip) = SLAB // RUN, divmod(W_LEAD, 3)
    ahead = lambda copies, r: (copies(r + lead) + copies(r + lead + 1))[skip:skip + 3]
    rest_a = [block(wm, 144 + i) for i in range(6)] + [block(w1, 48 + i) for i in (0, 4, 8)]
    rest_b = [block(w1, 48 + i) for i in (6, 10, 2, 7, 11, 3, 9, 1, 5)]
    second = (rest_b + over(first_b, 0, lead + 1))[:9 + W_LEAD]
    start([], second[:W_LEAD])
    start(rest_a + small[:1], second[W_LEAD:] + small[1:2])
    _loop(0, 24, lambda r: start(first_a(r), ahead(first_b, r)))
    for sel, col, width in ((sel_d, col_d, ND), (sel_f, col_f, NF)):
        sel[...] = _selector(width)
        for m in range(width):
            col[m] = _tile_coords(m, width, (8, LANE))[1] - _iota((8, LANE), 0)
    turn = nrun - lead - 1
    _loop(24, turn, lambda r: start(first_a(r), ahead(first_b, r)))
    start(over(first_a, turn, nrun), (first_b(nrun - 1) + over(second_b, 0, lead + 1))[skip:skip + 3 * (lead + 1)])
    start_second = lambda r: start(second_a(r), ahead(second_b, r))
    _loop(0, 16, start_second)
    for cp in small[:2]:
        cp().wait()
    _wait(wm_v, sem_w.at[0])

    c = _stack(c_v[...].astype(F32))
    moved = _dot((c * jax.nn.sigmoid(c)).astype(BF16), _selector(6 * ND))
    keep = []
    for m in range(6 * ND):
        column = out_row = _tile_coords(m, 6 * ND, (48, LANE))[1]
        for i in range(1, 6):
            out_row = jnp.where(column >= ND * i, out_row + 8 - ND, out_row)
        keep.append(out_row == _iota((48, LANE), 0))
    keep = jnp.concatenate(keep, axis=1)
    mod = jnp.zeros((48, LANE), F32)
    for j in range(ND):
        mod += _dot(jnp.where(keep, _row(moved, j, 48), 0.0).astype(BF16), wm_v[j * 6 * D:(j + 1) * 6 * D, :])
        _loop(16 + 5 * j, 21 + 5 * j, start_second)
    shift_a, scale_a, gate_a, shift_b, scale_b, gate_b = (mod[8 * i:8 * i + 8] for i in range(6))
    x0 = _stack(x_v[...].astype(F32))
    h = _layernorm(x0) * (1.0 + scale_a) + shift_a
    _loop(16 + 5 * ND, turn, start_second)
    start(over(second_a, turn, nrun) + small[2:],
          second_b(nrun - 1)[skip:] + (half_head(k_hbm, 0, 0, 1) + half_head(k_hbm, 0, 1, 1))[:LEAD])

    moved = _dot(h.astype(BF16), _selector(16))
    keep = ((_iota((16, 16 * LANE), 1) >> 3) & 15) == _iota((16, 16 * LANE), 0)
    lhs = jnp.concatenate([jnp.where(keep, _row(moved, j, 16), 0.0).astype(BF16) for j in range(ND)], axis=1)
    start_pair(k_hbm, 0)
    small[2]().wait()
    _wait(w1_v, sem_w.at[1])
    _wait(wq_v, sem_w.at[2])
    _wait(wo_v, sem_w.at[3])
    q = []
    for i in range(3):
        q.append(_dot(lhs, wq_v[:, i * LANE:(i + 1) * LANE, :].reshape(-1, LANE)))
        if i < 2:
            start_head(k_hbm, 1, i)
    q = jnp.concatenate(q, axis=0)
    row, lane = _iota((8, PAIR), 0), _iota((8, PAIR), 1)
    own = jnp.logical_or(jnp.logical_and(row == 0, lane < DH), jnp.logical_and(row == 1, lane >= DH))
    for p in range(NPAIR):
        q_s[p] = jnp.where(own, jnp.concatenate([_row(q, 3 * p + u) for u in range(3)], axis=1), 0.0)

    def scores(p):
        slot = slot_of(k_hbm, p)
        _wait(kv_v.at[slot], sem_kv.at[slot])
        s = _dot(q_s[p].astype(BF16), kv_v[slot]) * DH ** -0.5
        e = jnp.exp(s - jnp.max(s, axis=-1, keepdims=True))
        e_s[p] = e
        den_s[p] = jnp.broadcast_to(jnp.sum(e, axis=-1, keepdims=True), (8, LANE))

    last = NPAIR - 1
    scores(0)
    _loop(1, last - 1, lambda p: (start_pair(k_hbm, p + 1), scores(p)))
    start_head(k_hbm, last, 0, half_head(k_hbm, last, 1, 1) + half_head(v_hbm, 0, 0, 1))
    start_head(k_hbm, last, 1, half_head(v_hbm, 0, 0, 1) + half_head(v_hbm, 0, 1, 1))
    scores(last - 1)
    start_pair(v_hbm, 0)
    scores(last)

    def values(p, c0, c1):
        return lax.dot_general(e_s[p, :, c0:c1].astype(BF16), kv_v[slot_of(v_hbm, p), :, c0:c1],
                               (((1,), (1,)), ((), ())), preferred_element_type=F32)

    def left_operand(v, sel, col, rows):
        width = col.shape[0]
        g_s[:v.shape[0], :width * LANE] = _dot(v.astype(BF16), sel[...])

        def one(i, m):
            g = _row(g_s[i:i + 1, m * LANE:(m + 1) * LANE], 0)
            return jnp.concatenate([jnp.where(col[m] == r, g, 0.0) for r in range(0, rows, 8)], axis=0)

        return lambda blocks: jnp.concatenate([one(*divmod(b, width)).astype(BF16) for b in blocks], axis=1)

    def project(p, acc):
        o = jnp.where(own, acc / jnp.concatenate([den_s[p]] * 3, axis=1), 0.0)
        lhs = left_operand(_stack(jnp.sum(o, axis=0, keepdims=True)), sel_d, col_d, 8)(range(3 * ND))
        return _dot(lhs, wo_v[pl.ds(_aligned(p * ND * PAIR, ND * PAIR), ND * PAIR), :])

    def attend(p):
        slot = slot_of(v_hbm, p)
        _wait(kv_v.at[slot], sem_kv.at[slot])
        return project(p, values(p, 0, window))

    def v_step(p, att):
        start_pair(v_hbm, p + 1)
        return att + attend(p)

    att = lax.fori_loop(0, last - 2, v_step, jnp.zeros((8, LANE), F32))

    v_cols = [KV_COLS * n for n in _starts(V_GROUPS)]
    v_sem = lambda c: sem_v.at[sum(c >= e for e in v_cols[1:])]
    order = [ND * NF // 4 * n + s for s in range(ND * NF // 4) for n in (0, 2, 1, 3)]
    w2_at = _starts(W2_MXU + W2_VPU)
    w2 = [copy(w2_hbm.at[pl.ds(b * LANE, LANE)], w2_v.at[pl.ds(i * LANE, LANE)],
               sem_w2.at[sum(i >= e for e in w2_at[1:])]) for i, b in enumerate(order)]
    w2_second = w2[1:W2_BOTH:2] + w2[W2_BOTH:]
    last_low = half_head(v_hbm, last, 1, 1, v_sem)
    start_head(v_hbm, last - 1, 0)
    start_head(v_hbm, last - 1, 1, half_head(v_hbm, last, 0, 1) + last_low)
    att += attend(last - 2)
    start_head(v_hbm, last, 0, last_low + w2_second)
    start(half_head(v_hbm, last, 1, 0, v_sem), w2_second[LEAD - HALF:LEAD])
    att += attend(last - 1)
    start(w2[0:W2_BOTH:2], w2_second[LEAD:])
    slot = slot_of(v_hbm, last)
    _wait(kv_v.at[slot, pl.ds(0, DH)], sem_kv.at[slot])
    for i in range(len(V_GROUPS)):
        _wait(kv_v.at[slot, pl.ds(DH, DH), pl.ds(v_cols[i], v_cols[i + 1] - v_cols[i])], sem_v.at[i])
        acc_s[...] = values(last, v_cols[i], v_cols[i + 1]) + (acc_s[...] if i else 0.0)
    att += project(last, acc_s[...])

    x1 = x0 + gate_a * att
    h = _layernorm(x1) * (1.0 + scale_b) + shift_b
    bias = jnp.concatenate([b1_v[...].astype(F32), jnp.zeros((16 - NF, LANE), F32)], axis=0)
    act = _mish(_dot(left_operand(h, sel_f, col_f, 16)(range(ND * NF)), w1_v[...]) + bias)
    operand = left_operand(act, sel_d, col_d, 8)
    row, lane = _iota((8, LANE), 0), _iota((8, LANE), 1)
    tiles = [16 * b + i for b in order[sum(W2_MXU):] for i in range(16)]
    column = {}
    for n, t in enumerate(tiles):
        r, j = divmod(t, ND)
        if r not in column:
            column[r] = jnp.sum(jnp.where(lane == r % 16 * 8 + row, _row(act, r // 16), 0.0), axis=1, keepdims=True)
        a_s[n] = column[r] * gate_b[j:j + 1]
    y_s[...] = y = x1
    acc = [[] for _ in range(ND)]
    for i, (b0, b1) in enumerate(zip(w2_at, w2_at[1:])):
        rows = pl.ds(b0 * LANE, (b1 - b0) * LANE)
        _wait(w2_v.at[rows], sem_w2.at[i])
        if i < len(W2_MXU):
            y = y_s[...] + gate_b * _dot(operand(order[b0:b1]), w2_v[rows, :])
            if i < len(W2_MXU) - 1:
                y_s[...] = y
            continue
        w = w2_v[rows, :].astype(F32)
        for n in range(16 * (b1 - b0)):
            m = 16 * (b0 - sum(W2_MXU)) + n
            acc[tiles[m] % ND].append(w[8 * n:8 * n + 8] * a_s[m])
        if i == len(W2_MXU) + 1:
            for j in range(ND):
                acc[j].append(jnp.where(row == j, y, 0.0))
        for terms in acc:
            while len(terms) > 1:
                terms.insert(0, terms.pop() + terms.pop())
    for j in range(ND):
        o_ref[:, j * LANE:(j + 1) * LANE] = jnp.sum(acc[j][0], axis=0, keepdims=True).astype(o_ref.dtype)


@jax.jit
def pallas_adaLN_cond__sliding_block_cached__dense_activation_mish__decode_kernel(
    A_x: jax.Array,
    A_k_cache: jax.Array,
    A_v_cache: jax.Array,
    A_wq: jax.Array,
    A_wo: jax.Array,
    B_x: jax.Array,
    B_w1: jax.Array,
    B_b1: jax.Array,
    B_w2: jax.Array,
    c: jax.Array,
    w_mod: jax.Array,
):
    del B_x
    sk = A_k_cache.shape[2]
    window = min(4096, max(256, sk // 4))
    assert window == HALF // 3 * KV_COLS
    kt = jnp.swapaxes(A_k_cache, 2, 3).reshape(H * DH, sk)
    vt = jnp.swapaxes(A_v_cache, 2, 3).reshape(H * DH, sk)
    out = pl.pallas_call(
        _kernel,
        out_shape=jax.ShapeDtypeStruct((1, D), A_x.dtype),
        in_specs=[pl.BlockSpec(memory_space=pltpu.HBM)] * 10,
        out_specs=pl.BlockSpec(memory_space=pltpu.VMEM),
        scratch_shapes=[
            pltpu.VMEM((1, D), BF16),
            pltpu.VMEM((1, D), BF16),
            pltpu.VMEM((NF, LANE), BF16),
            pltpu.VMEM((6 * ND * D, LANE), BF16),
            pltpu.VMEM((D // 8, 3 * LANE, LANE), BF16),
            pltpu.VMEM((ND * H * DH, LANE), BF16),
            pltpu.VMEM((NF * D, LANE), BF16),
            pltpu.VMEM((ND * F, LANE), BF16),
            pltpu.VMEM((NSLOT, PAIR, window), BF16),
            pltpu.VMEM((NPAIR, 8, PAIR), F32),
            pltpu.VMEM((NPAIR, 8, window), F32),
            pltpu.VMEM((NPAIR, 8, LANE), F32),
            pltpu.VMEM((LANE, D), BF16),
            pltpu.VMEM((LANE, F), BF16),
            pltpu.VMEM((ND, 8, LANE), jnp.int32),
            pltpu.VMEM((NF, 8, LANE), jnp.int32),
            pltpu.VMEM((16, F), F32),
            pltpu.VMEM((8, PAIR), F32),
            pltpu.VMEM((8, LANE), F32),
            pltpu.VMEM((16 * sum(W2_VPU), 8, LANE), F32),
            pltpu.SemaphoreType.DMA((7,)),
            pltpu.SemaphoreType.DMA((NSLOT,)),
            pltpu.SemaphoreType.DMA((len(V_GROUPS),)),
            pltpu.SemaphoreType.DMA((len(W2_MXU + W2_VPU),)),
            pltpu.SemaphoreType.REGULAR,
        ],
        compiler_params=pltpu.CompilerParams(
            vmem_limit_bytes=64 * 2**20,
            disable_semaphore_checks=True,
        ),
        name="adaln_attn_mlp_decode",
    )(A_x.reshape(1, D), kt, vt, _tile_major(A_wq), _tile_major(A_wo), _tile_major(B_w1),
      B_b1.reshape(NF, LANE), _tile_major(B_w2), c, _tile_major(w_mod))
    return out.reshape(A_x.shape)
```

```python
import functools

import jax
import jax.numpy as jnp
from jax import lax
import jax.experimental.pallas as pl
import jax.experimental.pallas.tpu as pltpu

D = 640
H = 32
DH = 192
F = 1536
PAIR = 2 * DH
NPAIR = H // 2
LANE = 128
ND = D // LANE
NF = F // LANE
F32 = jnp.float32
BF16 = jnp.bfloat16

SLAB = 2048
RUN = 32
KV_ROWS, KV_COLS = 32, 512
HALF = 24
LEAD = 25
NSLOT = 3
V_GROUPS = (3, 2, 2, 1)
W2_MXU = (28, 20)
W2_VPU = (4, 4, 2, 1, 1)
W2_BOTH = 36


def _tile_major(w):
    r, c = w.shape
    return w.reshape(r // 8, 8, c // LANE, LANE).transpose(0, 2, 1, 3).reshape(-1, LANE)


def _iota(shape, dim):
    return lax.broadcasted_iota(jnp.int32, shape, dim)


def _row(v, i, rows=8):
    return jnp.broadcast_to(v[i:i + 1], (rows, v.shape[1]))


def _stack(v):
    out = jnp.zeros((8, LANE), F32)
    for j in range(v.shape[1] // LANE):
        out = jnp.where(_iota((8, LANE), 0) == j, _row(v[:, j * LANE:(j + 1) * LANE], 0), out)
    return out


def _tile_coords(block, width, shape):
    i = _iota(shape, 1) >> 3
    r0, c0 = divmod(16 * block, width)
    r, c = jnp.full(shape, r0, jnp.int32), i + c0
    for k in range(width - c0, 16, width):
        r = jnp.where(i >= k, r + 1, r)
        c = jnp.where(i >= k, c - width, c)
    return r, c


def _selector(width):
    shape = (LANE, LANE)
    source = lambda m: _tile_coords(m, width, shape)[0] * 8 + (_iota(shape, 1) & 7)
    return jnp.concatenate([jnp.where(source(m) == _iota(shape, 0), 1.0, 0.0).astype(BF16)
                            for m in range(width)], axis=1)


def _layernorm(x, eps=1e-5):
    total = lambda a: jnp.sum(jnp.sum(a, axis=1, keepdims=True), axis=0, keepdims=True)
    d = jnp.where(_iota(x.shape, 0) < ND, x - total(x) / D, 0.0)
    return d / jnp.sqrt(total(d * d) / D + eps)


def _mish(u):
    softplus = jnp.log1p(jnp.exp(-jnp.abs(u))) + jnp.where(u > 0, u, 0.0)
    return u * jnp.tanh(softplus)


def _dot(a, b):
    return jnp.dot(a, b, preferred_element_type=F32)


def _loop(lo, hi, body):
    lax.fori_loop(lo, hi, lambda i, carry: (body(i), carry)[1], 0)


def _aligned(i, n):
    return i if isinstance(i, int) else pl.multiple_of(i, n)


def _shuffled(i):
    return i ^ ((i & 1) << 1)


def _starts(sizes):
    return [sum(sizes[:i]) for i in range(len(sizes) + 1)]


def _wait(buf, sem):
    pltpu.make_async_copy(buf, buf, sem).wait()


def _kernel(x_hbm, k_hbm, v_hbm, wq_hbm, wo_hbm, w1_hbm, b1_hbm, w2_hbm, c_hbm, wm_hbm, o_hbm,
            o_ref, x_v, c_v, b1_v, wm_v, wq_v, wo_v, w1_v, w2_v, kv_v,
            q_s, e_s, den_s, sel_d, sel_f, col_d, col_f, g_s, acc_s, y_s, a_s,
            sem_w, sem_kv, sem_v, sem_w2, fence):
    window = kv_v.shape[-1]
    col0 = k_hbm.shape[1] - window
    copy = lambda src, dst, sem: functools.partial(pltpu.make_async_copy, src, dst, sem)

    def start(first, second):
        for i in range(max(len(first), len(second))):
            for queue, copies in enumerate((first, second)):
                if i < len(copies):
                    pl.semaphore_signal(fence, 1)
                    pl.semaphore_wait(fence, 1)
                    copies[i]().start(priority=queue)

    def runs(weight, slab, nslab, run):
        src, dst, sem = weight
        n = src.shape[0] // SLAB
        whole = lambda ref: ref if ref.shape[0] == n * SLAB else ref.at[pl.ds(0, n * SLAB)]
        at = (pl.ds(slab, nslab), pl.ds(_aligned(run * RUN, RUN), RUN))
        return copy(whole(src).reshape(n, SLAB, LANE).at[at], whole(dst).reshape(n, SLAB, LANE).at[at], sem)

    def piece(weight, row, nrow):
        src, dst, sem = weight
        return copy(src.at[pl.ds(row, nrow)], dst.at[pl.ds(row, nrow)], sem)

    def slot_of(src, p):
        return (p + (NPAIR if src is v_hbm else 0)) % NSLOT

    def half_head(src, p, which, half, sem_of=None):
        slot = slot_of(src, p)
        return [copy(src.at[pl.ds(_aligned(p * PAIR + r, KV_ROWS), KV_ROWS), pl.ds(col0 + c, KV_COLS)],
                     kv_v.at[slot, pl.ds(r, KV_ROWS), pl.ds(c, KV_COLS)],
                     sem_of(c) if sem_of else sem_kv.at[slot])
                for c in (KV_COLS * (i if sem_of else _shuffled(i)) for i in range(window // KV_COLS))
                for r in range(which * DH + (1 - half) * DH // 2, which * DH + (2 - half) * DH // 2, KV_ROWS)]

    def start_head(src, p, which, later=None):
        if later is None:
            later = half_head(src, p + which, 1 - which, 1) + half_head(src, p + 1, which, 1)
        start(half_head(src, p, which, 0), later[LEAD - HALF:LEAD])

    def start_pair(src, p):
        start_head(src, p, 0)
        start_head(src, p, 1)

    wm, w1 = (wm_hbm, wm_v, sem_w.at[0]), (w1_hbm, w1_v, sem_w.at[1])
    wq, wo = (wq_hbm, wq_v.reshape(wq_hbm.shape), sem_w.at[2]), (wo_hbm, wo_v, sem_w.at[3])
    small = [copy(s, d, sem_w.at[4 + i]) for i, (s, d) in enumerate(((c_hbm, c_v), (x_hbm, x_v), (b1_hbm, b1_v)))]
    first_a = lambda r: [runs(wm, s, 3, r) for s in (0, 3, 6)]
    first_b = lambda r: [runs(wq, 12, 3, r), runs(wo, 12, 3, r), runs(w1, 0, 3, r)]
    second_a = lambda r: [runs(wq, s, 4, r) for s in (0, 4, 8)]
    second_b = lambda r: [runs(wo, s, 4, r) for s in (0, 4, 8)]
    over = lambda copies, lo, hi: [cp for r in range(lo, hi) for cp in copies(r)]
    nrun, (lead, skip) = SLAB // RUN, divmod(LEAD, 3)
    ahead = lambda copies, r: (copies(r + lead) + copies(r + lead + 1))[skip:skip + 3]
    rest_a = [piece(wm, r, RUN) for r in range(9 * SLAB, wm_hbm.shape[0], RUN)]
    rest_a += [piece(w1, 3 * SLAB + i * LANE + r, RUN) for i in (0, 4) for r in range(0, LANE, RUN)]
    rest_a += [piece(w1, 3 * SLAB + 8 * LANE, LANE)]
    rest_b = [piece(w1, 3 * SLAB + i * LANE, LANE) for i in (6, 10, 2, 7, 11, 3, 9, 1, 5)]
    start(rest_a + small[:2], (rest_b + over(first_b, 0, lead + 1))[:9 + LEAD] + small[2:])
    _loop(0, 24, lambda r: start(first_a(r), ahead(first_b, r)))
    for sel, col, width in ((sel_d, col_d, ND), (sel_f, col_f, NF)):
        sel[...] = _selector(width)
        for m in range(width):
            col[m] = _tile_coords(m, width, (8, LANE))[1] - _iota((8, LANE), 0)
    turn = nrun - lead - 1
    _loop(24, turn, lambda r: start(first_a(r), ahead(first_b, r)))
    start(over(first_a, turn, nrun), (first_b(nrun - 1) + over(second_b, 0, lead + 1))[skip:skip + 3 * (lead + 1)])
    start_second = lambda r: start(second_a(r), ahead(second_b, r))
    _loop(0, 16, start_second)
    for cp in small:
        cp().wait()
    _wait(wm_v, sem_w.at[0])

    c = _stack(c_v[...].astype(F32))
    moved = _dot((c * jax.nn.sigmoid(c)).astype(BF16), _selector(6 * ND))
    keep = []
    for m in range(6 * ND):
        column = out_row = _tile_coords(m, 6 * ND, (48, LANE))[1]
        for i in range(1, 6):
            out_row = jnp.where(column >= ND * i, out_row + 8 - ND, out_row)
        keep.append(out_row == _iota((48, LANE), 0))
    keep = jnp.concatenate(keep, axis=1)
    mod = jnp.zeros((48, LANE), F32)
    for j in range(ND):
        mod += _dot(jnp.where(keep, _row(moved, j, 48), 0.0).astype(BF16), wm_v[j * 6 * D:(j + 1) * 6 * D, :])
        _loop(16 + 5 * j, 21 + 5 * j, start_second)
    shift_a, scale_a, gate_a, shift_b, scale_b, gate_b = (mod[8 * i:8 * i + 8] for i in range(6))
    x0 = _stack(x_v[...].astype(F32))
    h = _layernorm(x0) * (1.0 + scale_a) + shift_a
    _loop(16 + 5 * ND, turn, start_second)
    start(over(second_a, turn, nrun),
          second_b(nrun - 1)[skip:] + (half_head(k_hbm, 0, 0, 1) + half_head(k_hbm, 0, 1, 1))[:LEAD])

    moved = _dot(h.astype(BF16), _selector(16))
    keep = ((_iota((16, 16 * LANE), 1) >> 3) & 15) == _iota((16, 16 * LANE), 0)
    lhs = jnp.concatenate([jnp.where(keep, _row(moved, j, 16), 0.0).astype(BF16) for j in range(ND)], axis=1)
    start_pair(k_hbm, 0)
    _wait(w1_v, sem_w.at[1])
    _wait(wq_v, sem_w.at[2])
    _wait(wo_v, sem_w.at[3])
    q = []
    for i in range(3):
        q.append(_dot(lhs, wq_v[:, i * LANE:(i + 1) * LANE, :].reshape(-1, LANE)))
        if i < 2:
            start_head(k_hbm, 1, i)
    q = jnp.concatenate(q, axis=0)
    row, lane = _iota((8, PAIR), 0), _iota((8, PAIR), 1)
    own = jnp.logical_or(jnp.logical_and(row == 0, lane < DH), jnp.logical_and(row == 1, lane >= DH))
    for p in range(NPAIR):
        q_s[p] = jnp.where(own, jnp.concatenate([_row(q, 3 * p + u) for u in range(3)], axis=1), 0.0)

    def scores(p):
        slot = slot_of(k_hbm, p)
        _wait(kv_v.at[slot], sem_kv.at[slot])
        s = _dot(q_s[p].astype(BF16), kv_v[slot]) * DH ** -0.5
        e = jnp.exp(s - jnp.max(s, axis=-1, keepdims=True))
        e_s[p] = e
        den_s[p] = jnp.broadcast_to(jnp.sum(e, axis=-1, keepdims=True), (8, LANE))

    last = NPAIR - 1
    scores(0)
    _loop(1, last - 1, lambda p: (start_pair(k_hbm, p + 1), scores(p)))
    start_head(k_hbm, last, 0, half_head(k_hbm, last, 1, 1) + half_head(v_hbm, 0, 0, 1))
    start_head(k_hbm, last, 1, half_head(v_hbm, 0, 0, 1) + half_head(v_hbm, 0, 1, 1))
    scores(last - 1)
    start_pair(v_hbm, 0)
    scores(last)

    def values(p, c0, c1):
        return lax.dot_general(e_s[p, :, c0:c1].astype(BF16), kv_v[slot_of(v_hbm, p), :, c0:c1],
                               (((1,), (1,)), ((), ())), preferred_element_type=F32)

    def left_operand(v, sel, col, rows):
        width = col.shape[0]
        g_s[:v.shape[0], :width * LANE] = _dot(v.astype(BF16), sel[...])

        def one(i, m):
            g = _row(g_s[i:i + 1, m * LANE:(m + 1) * LANE], 0)
            return jnp.concatenate([jnp.where(col[m] == r, g, 0.0) for r in range(0, rows, 8)], axis=0)

        return lambda blocks: jnp.concatenate([one(*divmod(b, width)).astype(BF16) for b in blocks], axis=1)

    def project(p, acc):
        o = jnp.where(own, acc / jnp.concatenate([den_s[p]] * 3, axis=1), 0.0)
        lhs = left_operand(_stack(jnp.sum(o, axis=0, keepdims=True)), sel_d, col_d, 8)(range(3 * ND))
        return _dot(lhs, wo_v[pl.ds(_aligned(p * ND * PAIR, ND * PAIR), ND * PAIR), :])

    def attend(p):
        slot = slot_of(v_hbm, p)
        _wait(kv_v.at[slot], sem_kv.at[slot])
        return project(p, values(p, 0, window))

    def v_step(p, att):
        start_pair(v_hbm, p + 1)
        return att + attend(p)

    att = lax.fori_loop(0, last - 2, v_step, jnp.zeros((8, LANE), F32))

    v_cols = [KV_COLS * n for n in _starts(V_GROUPS)]
    v_sem = lambda c: sem_v.at[sum(c >= e for e in v_cols[1:])]
    order = [ND * NF // 4 * n + s for s in range(ND * NF // 4) for n in (0, 2, 1, 3)]
    w2_at = _starts(W2_MXU + W2_VPU)
    w2 = [copy(w2_hbm.at[pl.ds(b * LANE, LANE)], w2_v.at[pl.ds(i * LANE, LANE)],
               sem_w2.at[sum(i >= e for e in w2_at[1:])]) for i, b in enumerate(order)]
    w2_second = w2[1:W2_BOTH:2] + w2[W2_BOTH:]
    last_half = half_head(v_hbm, last, 1, 1, v_sem)
    start_head(v_hbm, last - 1, 0)
    start_head(v_hbm, last - 1, 1, half_head(v_hbm, last, 0, 1) + last_half)
    att += attend(last - 2)
    start_head(v_hbm, last, 0, last_half + w2_second)
    start(half_head(v_hbm, last, 1, 0, v_sem), w2_second[LEAD - HALF:LEAD])
    att += attend(last - 1)
    start(w2[0:W2_BOTH:2], w2_second[LEAD:])
    slot = slot_of(v_hbm, last)
    _wait(kv_v.at[slot, pl.ds(0, DH)], sem_kv.at[slot])
    for i in range(len(V_GROUPS)):
        _wait(kv_v.at[slot, pl.ds(DH, DH), pl.ds(v_cols[i], v_cols[i + 1] - v_cols[i])], sem_v.at[i])
        acc_s[...] = values(last, v_cols[i], v_cols[i + 1]) + (acc_s[...] if i else 0.0)
    att += project(last, acc_s[...])

    x1 = x0 + gate_a * att
    h = _layernorm(x1) * (1.0 + scale_b) + shift_b
    bias = jnp.concatenate([b1_v[...].astype(F32), jnp.zeros((16 - NF, LANE), F32)], axis=0)
    act = _mish(_dot(left_operand(h, sel_f, col_f, 16)(range(ND * NF)), w1_v[...]) + bias)
    operand = left_operand(act, sel_d, col_d, 8)
    row, lane = _iota((8, LANE), 0), _iota((8, LANE), 1)
    tiles = [16 * b + i for b in order[sum(W2_MXU):] for i in range(16)]
    column = {}
    for n, t in enumerate(tiles):
        r, j = divmod(t, ND)
        if r not in column:
            column[r] = jnp.sum(jnp.where(lane == r % 16 * 8 + row, _row(act, r // 16), 0.0), axis=1, keepdims=True)
        a_s[n] = column[r] * gate_b[j:j + 1]
    y_s[...] = y = x1
    acc = [[] for _ in range(ND)]
    for i, (b0, b1) in enumerate(zip(w2_at, w2_at[1:])):
        rows = pl.ds(b0 * LANE, (b1 - b0) * LANE)
        _wait(w2_v.at[rows], sem_w2.at[i])
        if i < len(W2_MXU):
            y = y_s[...] + gate_b * _dot(operand(order[b0:b1]), w2_v[rows, :])
            if i < len(W2_MXU) - 1:
                y_s[...] = y
            continue
        w = w2_v[rows, :].astype(F32)
        for n in range(16 * (b1 - b0)):
            m = 16 * (b0 - sum(W2_MXU)) + n
            acc[tiles[m] % ND].append(w[8 * n:8 * n + 8] * a_s[m])
        if i == len(W2_MXU) + 1:
            for j in range(ND):
                acc[j].append(jnp.where(row == j, y, 0.0))
        for terms in acc:
            while len(terms) > 1:
                terms.insert(0, terms.pop() + terms.pop())
    for j in range(ND):
        o_ref[:, j * LANE:(j + 1) * LANE] = jnp.sum(acc[j][0], axis=0, keepdims=True).astype(o_ref.dtype)
    out = pltpu.make_async_copy(o_ref, o_hbm, sem_w.at[7])
    out.start()
    out.wait()


@jax.jit
def pallas_adaLN_cond__sliding_block_cached__dense_activation_mish__decode_kernel(
    A_x: jax.Array,
    A_k_cache: jax.Array,
    A_v_cache: jax.Array,
    A_wq: jax.Array,
    A_wo: jax.Array,
    B_x: jax.Array,
    B_w1: jax.Array,
    B_b1: jax.Array,
    B_w2: jax.Array,
    c: jax.Array,
    w_mod: jax.Array,
):
    del B_x
    sk = A_k_cache.shape[2]
    window = min(4096, max(256, sk // 4))
    assert window == HALF // 3 * KV_COLS
    kt = jnp.swapaxes(A_k_cache, 2, 3).reshape(H * DH, sk)
    vt = jnp.swapaxes(A_v_cache, 2, 3).reshape(H * DH, sk)
    out = pl.pallas_call(
        _kernel,
        out_shape=jax.ShapeDtypeStruct((1, D), A_x.dtype),
        in_specs=[pl.BlockSpec(memory_space=pltpu.HBM)] * 10,
        out_specs=pl.BlockSpec(memory_space=pltpu.HBM),
        scratch_shapes=[
            pltpu.VMEM((1, D), BF16),
            pltpu.VMEM((1, D), BF16),
            pltpu.VMEM((1, D), BF16),
            pltpu.VMEM((NF, LANE), BF16),
            pltpu.VMEM((6 * ND * D, LANE), BF16),
            pltpu.VMEM((D // 8, 3 * LANE, LANE), BF16),
            pltpu.VMEM((ND * H * DH, LANE), BF16),
            pltpu.VMEM((NF * D, LANE), BF16),
            pltpu.VMEM((ND * F, LANE), BF16),
            pltpu.VMEM((NSLOT, PAIR, window), BF16),
            pltpu.VMEM((NPAIR, 8, PAIR), F32),
            pltpu.VMEM((NPAIR, 8, window), F32),
            pltpu.VMEM((NPAIR, 8, LANE), F32),
            pltpu.VMEM((LANE, D), BF16),
            pltpu.VMEM((LANE, F), BF16),
            pltpu.VMEM((ND, 8, LANE), jnp.int32),
            pltpu.VMEM((NF, 8, LANE), jnp.int32),
            pltpu.VMEM((16, F), F32),
            pltpu.VMEM((8, PAIR), F32),
            pltpu.VMEM((8, LANE), F32),
            pltpu.VMEM((16 * sum(W2_VPU), 8, LANE), F32),
            pltpu.SemaphoreType.DMA((8,)),
            pltpu.SemaphoreType.DMA((NSLOT,)),
            pltpu.SemaphoreType.DMA((len(V_GROUPS),)),
            pltpu.SemaphoreType.DMA((len(W2_MXU + W2_VPU),)),
            pltpu.SemaphoreType.REGULAR,
        ],
        compiler_params=pltpu.CompilerParams(
            vmem_limit_bytes=64 * 2**20,
            disable_semaphore_checks=True,
        ),
        name="adaln_attn_mlp_decode",
    )(A_x.reshape(1, D), kt, vt, _tile_major(A_wq), _tile_major(A_wo), _tile_major(B_w1),
      B_b1.reshape(NF, LANE), _tile_major(B_w2), c, _tile_major(w_mod))
    return out.reshape(A_x.shape)
```

```python
import functools

import jax
import jax.numpy as jnp
from jax import lax
import jax.experimental.pallas as pl
import jax.experimental.pallas.tpu as pltpu

D = 640
H = 32
DH = 192
F = 1536
PAIR = 2 * DH
NPAIR = H // 2
LANE = 128
ND = D // LANE
NF = F // LANE
F32 = jnp.float32
BF16 = jnp.bfloat16

SLAB = 2048
RUN = 32
KV_ROWS, KV_COLS = 32, 512
HALF = 24
LEAD = 25
PITCH = 32
NSLOT = 3
V_GROUPS = (3, 2, 2, 1)
W2_MXU = (28, 20)
W2_VPU = (4, 4, 2, 1, 1)
W2_BOTH = 36


def _tile_major(w):
    r, c = w.shape
    return w.reshape(r // 8, 8, c // LANE, LANE).transpose(0, 2, 1, 3).reshape(-1, LANE)


def _iota(shape, dim):
    return lax.broadcasted_iota(jnp.int32, shape, dim)


def _row(v, i, rows=8):
    return jnp.broadcast_to(v[i:i + 1], (rows, v.shape[1]))


def _stack(v):
    out = jnp.zeros((8, LANE), F32)
    for j in range(v.shape[1] // LANE):
        out = jnp.where(_iota((8, LANE), 0) == j, _row(v[:, j * LANE:(j + 1) * LANE], 0), out)
    return out


def _tile_coords(block, width, shape):
    i = _iota(shape, 1) >> 3
    r0, c0 = divmod(16 * block, width)
    r, c = jnp.full(shape, r0, jnp.int32), i + c0
    for k in range(width - c0, 16, width):
        r = jnp.where(i >= k, r + 1, r)
        c = jnp.where(i >= k, c - width, c)
    return r, c


def _selector(width):
    shape = (LANE, LANE)
    source = lambda m: _tile_coords(m, width, shape)[0] * 8 + (_iota(shape, 1) & 7)
    return jnp.concatenate([jnp.where(source(m) == _iota(shape, 0), 1.0, 0.0).astype(BF16)
                            for m in range(width)], axis=1)


def _layernorm(x, eps=1e-5):
    total = lambda a: jnp.sum(jnp.sum(a, axis=1, keepdims=True), axis=0, keepdims=True)
    d = jnp.where(_iota(x.shape, 0) < ND, x - total(x) / D, 0.0)
    return d / jnp.sqrt(total(d * d) / D + eps)


def _mish(u):
    softplus = jnp.log1p(jnp.exp(-jnp.abs(u))) + jnp.where(u > 0, u, 0.0)
    return u * jnp.tanh(softplus)


def _dot(a, b):
    return jnp.dot(a, b, preferred_element_type=F32)


def _loop(lo, hi, body):
    lax.fori_loop(lo, hi, lambda i, carry: (body(i), carry)[1], 0)


def _aligned(i, n):
    return i if isinstance(i, int) else pl.multiple_of(i, n)


def _shuffled(i):
    return i ^ ((i & 1) << 1)


def _starts(sizes):
    return [sum(sizes[:i]) for i in range(len(sizes) + 1)]


def _wait(buf, sem):
    pltpu.make_async_copy(buf, buf, sem).wait()


def _kernel(x_hbm, k_hbm, v_hbm, wq_hbm, wo_hbm, w1_hbm, b1_hbm, w2_hbm, c_hbm, wm_hbm, o_hbm,
            o_v, x_v, c_v, b1_v, wm_v, wq_v, wo_v, w1_v, w2_v, kv_v,
            q_s, e_s, den_s, sel_d, sel_f, col_d, col_f, g_s, acc_s, y_s, a_s,
            sem_w, sem_kv, sem_v, sem_w2, fence):
    window = kv_v.shape[-1]
    col0 = k_hbm.shape[1] - window
    copy = lambda src, dst, sem: functools.partial(pltpu.make_async_copy, src, dst, sem)

    def start(first, second):
        for i in range(max(len(first), len(second))):
            for queue, copies in enumerate((first, second)):
                if i < len(copies):
                    pl.semaphore_signal(fence, 1)
                    pl.semaphore_wait(fence, 1)
                    copies[i]().start(priority=queue)

    def slot_of(src, p):
        return (p + (NPAIR if src is v_hbm else 0)) % NSLOT

    def half_head(src, p, which, half, sem_of=None):
        slot = slot_of(src, p)
        return [copy(src.at[pl.ds(_aligned(p * PAIR + r, KV_ROWS), KV_ROWS), pl.ds(col0 + c, KV_COLS)],
                     kv_v.at[slot, pl.ds(r, KV_ROWS), pl.ds(c, KV_COLS)],
                     sem_of(c) if sem_of else sem_kv.at[slot])
                for c in (KV_COLS * (i if sem_of else _shuffled(i)) for i in range(window // KV_COLS))
                for r in range(which * DH + (1 - half) * DH // 2, which * DH + (2 - half) * DH // 2, KV_ROWS)]

    def start_head(src, p, which, later=None):
        if later is None:
            later = half_head(src, p + which, 1 - which, 1) + half_head(src, p + 1, which, 1)
        start(half_head(src, p, which, 0), later[LEAD - HALF:LEAD])

    def start_pair(src, p):
        start_head(src, p, 0)
        start_head(src, p, 1)

    def runs(weight, slab, nslab, run):
        src, dst, sem = weight
        at = (pl.ds(slab, nslab), pl.ds(_aligned(run * RUN, RUN), RUN))
        return copy(src.at[at], dst.at[at], sem)

    def blocks(ref, ids):
        per = SLAB // LANE
        return jnp.concatenate([ref[b // per, pl.ds(_aligned(b % per * LANE, LANE), LANE), :] for b in ids], axis=0)

    spots = [(w, b) for first in range(PITCH)
             for w in ((wm_hbm, wm_v, sem_w.at[0]), (w1_hbm, w1_v, sem_w.at[1]))
             for b in range(first, w[0].shape[0] // LANE, PITCH)]
    pieces = lambda spots, n: [copy(src.at[pl.ds(r, n)], dst.at[pl.ds(r, n)], sem)
                               for (src, dst, sem), b in spots for r in range(b * LANE, (b + 1) * LANE, n)]
    small = [copy(s, d, sem_w.at[4 + i]) for i, (s, d) in enumerate(((c_hbm, c_v), (x_hbm, x_v), (b1_hbm, b1_v)))]
    wq, wo = (wq_hbm, wq_v, sem_w.at[2]), (wo_hbm, wo_v, sem_w.at[3])
    first = lambda r: [runs(wq, s, 4, r) for s in (0, 4, 8)]
    second_a = lambda r: [runs(wq, 12, 3, r), runs(wo, 0, 3, r), runs(wo, 3, 3, r)]
    second_b = lambda r: [runs(wo, s, 3, r) for s in (6, 9, 12)]
    over = lambda copies, lo, hi: [cp for r in range(lo, hi) for cp in copies(r)]
    nrun, (lead, skip) = SLAB // RUN, divmod(LEAD, 3)
    other = pieces(spots[1:18:2], LANE) + over(first, 0, nrun) + over(second_b, 0, lead + 1)
    start(pieces(spots[0:16:2], RUN) + small[:2] + pieces(spots[16:17] + spots[18:], LANE),
          other[:32] + small[2:] + other[32:len(other) - 3 + skip])
    start_runs = lambda r: start(second_a(r), (second_b(r + lead) + second_b(r + lead + 1))[skip:skip + 3])
    turn = nrun - lead - 1
    _loop(0, 8, start_runs)
    for sel, col, width in ((sel_d, col_d, ND), (sel_f, col_f, NF)):
        sel[...] = _selector(width)
        for m in range(width):
            col[m] = _tile_coords(m, width, (8, LANE))[1] - _iota((8, LANE), 0)
    _loop(8, 16, start_runs)
    for cp in small:
        cp().wait()
    _wait(wm_v, sem_w.at[0])
    _wait(w1_v, sem_w.at[1])

    c = _stack(c_v[...].astype(F32))
    moved = _dot((c * jax.nn.sigmoid(c)).astype(BF16), _selector(6 * ND))
    keep = []
    for m in range(6 * ND):
        column = out_row = _tile_coords(m, 6 * ND, (48, LANE))[1]
        for i in range(1, 6):
            out_row = jnp.where(column >= ND * i, out_row + 8 - ND, out_row)
        keep.append(out_row == _iota((48, LANE), 0))
    keep = jnp.concatenate(keep, axis=1)
    mod = jnp.zeros((48, LANE), F32)
    for j in range(ND):
        mod += _dot(jnp.where(keep, _row(moved, j, 48), 0.0).astype(BF16), wm_v[j * 6 * D:(j + 1) * 6 * D, :])
        _loop(16 + 6 * j, 22 + 6 * j, start_runs)
    shift_a, scale_a, gate_a, shift_b, scale_b, gate_b = (mod[8 * i:8 * i + 8] for i in range(6))
    x0 = _stack(x_v[...].astype(F32))
    h = _layernorm(x0) * (1.0 + scale_a) + shift_a
    _loop(16 + 6 * ND, turn, start_runs)
    start(over(second_a, turn, nrun), second_b(nrun - 1)[skip:] + (half_head(k_hbm, 0, 0, 1) + half_head(k_hbm, 0, 1, 1))[:LEAD])

    moved = _dot(h.astype(BF16), _selector(16))
    keep = ((_iota((16, 16 * LANE), 1) >> 3) & 15) == _iota((16, 16 * LANE), 0)
    lhs = jnp.concatenate([jnp.where(keep, _row(moved, j, 16), 0.0).astype(BF16) for j in range(ND)], axis=1)
    start_pair(k_hbm, 0)
    _wait(wq_v, sem_w.at[2])
    _wait(wo_v, sem_w.at[3])
    q = []
    for i in range(3):
        q.append(_dot(lhs, blocks(wq_v, range(i, 3 * D // 8, 3))))
        if i < 2:
            start_head(k_hbm, 1, i)
    q = jnp.concatenate(q, axis=0)
    row, lane = _iota((8, PAIR), 0), _iota((8, PAIR), 1)
    own = jnp.logical_or(jnp.logical_and(row == 0, lane < DH), jnp.logical_and(row == 1, lane >= DH))
    for p in range(NPAIR):
        q_s[p] = jnp.where(own, jnp.concatenate([_row(q, 3 * p + u) for u in range(3)], axis=1), 0.0)

    def scores(p):
        slot = slot_of(k_hbm, p)
        _wait(kv_v.at[slot], sem_kv.at[slot])
        s = _dot(q_s[p].astype(BF16), kv_v[slot]) * DH ** -0.5
        e = jnp.exp(s - jnp.max(s, axis=-1, keepdims=True))
        e_s[p] = e
        den_s[p] = jnp.broadcast_to(jnp.sum(e, axis=-1, keepdims=True), (8, LANE))

    last = NPAIR - 1
    scores(0)
    _loop(1, last - 1, lambda p: (start_pair(k_hbm, p + 1), scores(p)))
    start_head(k_hbm, last, 0, half_head(k_hbm, last, 1, 1) + half_head(v_hbm, 0, 0, 1))
    start_head(k_hbm, last, 1, half_head(v_hbm, 0, 0, 1) + half_head(v_hbm, 0, 1, 1))
    scores(last - 1)
    start_pair(v_hbm, 0)
    scores(last)

    def values(p, c0, c1):
        return lax.dot_general(e_s[p, :, c0:c1].astype(BF16), kv_v[slot_of(v_hbm, p), :, c0:c1],
                               (((1,), (1,)), ((), ())), preferred_element_type=F32)

    def left_operand(v, sel, col, rows):
        width = col.shape[0]
        g_s[:v.shape[0], :width * LANE] = _dot(v.astype(BF16), sel[...])

        def one(i, m):
            g = _row(g_s[i:i + 1, m * LANE:(m + 1) * LANE], 0)
            return jnp.concatenate([jnp.where(col[m] == r, g, 0.0) for r in range(0, rows, 8)], axis=0)

        return lambda blocks: jnp.concatenate([one(*divmod(b, width)).astype(BF16) for b in blocks], axis=1)

    def project(p, acc):
        o = jnp.where(own, acc / jnp.concatenate([den_s[p]] * 3, axis=1), 0.0)
        lhs = left_operand(_stack(jnp.sum(o, axis=0, keepdims=True)), sel_d, col_d, 8)(range(3 * ND))
        return _dot(lhs, blocks(wo_v, [p * 3 * ND + b for b in range(3 * ND)]))

    def attend(p):
        slot = slot_of(v_hbm, p)
        _wait(kv_v.at[slot], sem_kv.at[slot])
        return project(p, values(p, 0, window))

    def v_step(p, att):
        start_pair(v_hbm, p + 1)
        return att + attend(p)

    att = lax.fori_loop(0, last - 2, v_step, jnp.zeros((8, LANE), F32))

    v_cols = [KV_COLS * n for n in _starts(V_GROUPS)]
    v_sem = lambda c: sem_v.at[sum(c >= e for e in v_cols[1:])]
    order = [ND * NF // 4 * n + s for s in range(ND * NF // 4) for n in (0, 2, 1, 3)]
    w2_at = _starts(W2_MXU + W2_VPU)
    w2 = [copy(w2_hbm.at[pl.ds(b * LANE, LANE)], w2_v.at[pl.ds(i * LANE, LANE)],
               sem_w2.at[sum(i >= e for e in w2_at[1:])]) for i, b in enumerate(order)]
    w2_second = w2[1:W2_BOTH:2] + w2[W2_BOTH:]
    last_half = half_head(v_hbm, last, 1, 1, v_sem)
    start_head(v_hbm, last - 1, 0)
    start_head(v_hbm, last - 1, 1, half_head(v_hbm, last, 0, 1) + last_half)
    att += attend(last - 2)
    start_head(v_hbm, last, 0, last_half + w2_second)
    start(half_head(v_hbm, last, 1, 0, v_sem), w2_second[LEAD - HALF:LEAD])
    att += attend(last - 1)
    start(w2[0:W2_BOTH:2], w2_second[LEAD:])
    slot = slot_of(v_hbm, last)
    _wait(kv_v.at[slot, pl.ds(0, DH)], sem_kv.at[slot])
    for i in range(len(V_GROUPS)):
        _wait(kv_v.at[slot, pl.ds(DH, DH), pl.ds(v_cols[i], v_cols[i + 1] - v_cols[i])], sem_v.at[i])
        acc_s[...] = values(last, v_cols[i], v_cols[i + 1]) + (acc_s[...] if i else 0.0)
    att += project(last, acc_s[...])

    x1 = x0 + gate_a * att
    h = _layernorm(x1) * (1.0 + scale_b) + shift_b
    bias = jnp.concatenate([b1_v[...].astype(F32), jnp.zeros((16 - NF, LANE), F32)], axis=0)
    act = _mish(_dot(left_operand(h, sel_f, col_f, 16)(range(ND * NF)), w1_v[...]) + bias)
    operand = left_operand(act, sel_d, col_d, 8)
    row, lane = _iota((8, LANE), 0), _iota((8, LANE), 1)
    tiles = [16 * b + i for b in order[sum(W2_MXU):] for i in range(16)]
    column = {}
    for n, t in enumerate(tiles):
        r, j = divmod(t, ND)
        if r not in column:
            column[r] = jnp.sum(jnp.where(lane == r % 16 * 8 + row, _row(act, r // 16), 0.0), axis=1, keepdims=True)
        a_s[n] = column[r] * gate_b[j:j + 1]
    y_s[...] = y = x1
    acc = [[] for _ in range(ND)]
    for i, (b0, b1) in enumerate(zip(w2_at, w2_at[1:])):
        rows = pl.ds(b0 * LANE, (b1 - b0) * LANE)
        _wait(w2_v.at[rows], sem_w2.at[i])
        if i < len(W2_MXU):
            y = y_s[...] + gate_b * _dot(operand(order[b0:b1]), w2_v[rows, :])
            if i < len(W2_MXU) - 1:
                y_s[...] = y
            continue
        w = w2_v[rows, :].astype(F32)
        for n in range(16 * (b1 - b0)):
            m = 16 * (b0 - sum(W2_MXU)) + n
            acc[tiles[m] % ND].append(w[8 * n:8 * n + 8] * a_s[m])
        if i == len(W2_MXU) + 1:
            for j in range(ND):
                acc[j].append(jnp.where(row == j, y, 0.0))
        for terms in acc:
            while len(terms) > 1:
                terms.insert(0, terms.pop() + terms.pop())
    for j in range(ND):
        o_v[:, j * LANE:(j + 1) * LANE] = jnp.sum(acc[j][0], axis=0, keepdims=True).astype(o_v.dtype)
    out = pltpu.make_async_copy(o_v, o_hbm, sem_w.at[7])
    out.start()
    out.wait()


@jax.jit
def pallas_adaLN_cond__sliding_block_cached__dense_activation_mish__decode_kernel(
    A_x: jax.Array,
    A_k_cache: jax.Array,
    A_v_cache: jax.Array,
    A_wq: jax.Array,
    A_wo: jax.Array,
    B_x: jax.Array,
    B_w1: jax.Array,
    B_b1: jax.Array,
    B_w2: jax.Array,
    c: jax.Array,
    w_mod: jax.Array,
):
    del B_x
    sk = A_k_cache.shape[2]
    window = min(4096, max(256, sk // 4))
    assert window == HALF // 3 * KV_COLS
    kt = jnp.swapaxes(A_k_cache, 2, 3).reshape(H * DH, sk)
    vt = jnp.swapaxes(A_v_cache, 2, 3).reshape(H * DH, sk)
    slabs = (ND * H * DH // SLAB, SLAB, LANE)
    out = pl.pallas_call(
        _kernel,
        out_shape=jax.ShapeDtypeStruct((1, D), A_x.dtype),
        in_specs=[pl.BlockSpec(memory_space=pltpu.HBM)] * 10,
        out_specs=pl.BlockSpec(memory_space=pltpu.HBM),
        scratch_shapes=[
            pltpu.VMEM((1, D), BF16),
            pltpu.VMEM((1, D), BF16),
            pltpu.VMEM((1, D), BF16),
            pltpu.VMEM((NF, LANE), BF16),
            pltpu.VMEM((6 * ND * D, LANE), BF16),
            pltpu.VMEM(slabs, BF16),
            pltpu.VMEM(slabs, BF16),
            pltpu.VMEM((NF * D, LANE), BF16),
            pltpu.VMEM((ND * F, LANE), BF16),
            pltpu.VMEM((NSLOT, PAIR, window), BF16),
            pltpu.VMEM((NPAIR, 8, PAIR), F32),
            pltpu.VMEM((NPAIR, 8, window), F32),
            pltpu.VMEM((NPAIR, 8, LANE), F32),
            pltpu.VMEM((LANE, D), BF16),
            pltpu.VMEM((LANE, F), BF16),
            pltpu.VMEM((ND, 8, LANE), jnp.int32),
            pltpu.VMEM((NF, 8, LANE), jnp.int32),
            pltpu.VMEM((16, F), F32),
            pltpu.VMEM((8, PAIR), F32),
            pltpu.VMEM((8, LANE), F32),
            pltpu.VMEM((16 * sum(W2_VPU), 8, LANE), F32),
            pltpu.SemaphoreType.DMA((8,)),
            pltpu.SemaphoreType.DMA((NSLOT,)),
            pltpu.SemaphoreType.DMA((len(V_GROUPS),)),
            pltpu.SemaphoreType.DMA((len(W2_MXU + W2_VPU),)),
            pltpu.SemaphoreType.REGULAR,
        ],
        compiler_params=pltpu.CompilerParams(
            vmem_limit_bytes=64 * 2**20,
            disable_semaphore_checks=True,
        ),
        name="adaln_attn_mlp_decode",
    )(A_x.reshape(1, D), kt, vt, _tile_major(A_wq).reshape(slabs), _tile_major(A_wo).reshape(slabs),
      _tile_major(B_w1), B_b1.reshape(NF, LANE), _tile_major(B_w2), c, _tile_major(w_mod))
    return out.reshape(A_x.shape)
```

```python
import functools

import jax
import jax.numpy as jnp
from jax import lax
import jax.experimental.pallas as pl
import jax.experimental.pallas.tpu as pltpu

D = 640
H = 32
DH = 192
F = 1536
PAIR = 2 * DH
NPAIR = H // 2
LANE = 128
F32 = jnp.float32
BF16 = jnp.bfloat16

RUN = 32
KV_ROWS, KV_COLS = 32, 512
NSLOT = 3
V_LAST = (3, 2, 2, 1)
W2_BOTH = 44
W2_STEPS = (7, 3, 2, 2, 1)


def _tile_major(w, slabs):
    r, c = w.shape
    return w.reshape(r // 8, 8, c // LANE, LANE).transpose(0, 2, 1, 3).reshape(slabs, -1, LANE)


def _iota(shape, dim):
    return lax.broadcasted_iota(jnp.int32, shape, dim)


def _rows(v, n):
    row = _iota((8, LANE), 0)
    out = jnp.zeros((8, LANE), F32)
    for j in range(n):
        out = jnp.where(row == j, jnp.broadcast_to(v[:, j * LANE:(j + 1) * LANE], (8, LANE)), out)
    return out


def _tile_coords(t0, width, shape, run=16):
    i = (_iota(shape, 1) >> 3) & (run - 1)
    r = jnp.full(shape, t0 // width, jnp.int32)
    c = i + t0 % width
    for k in range(width - t0 % width, run, width):
        r = jnp.where(i >= k, r + 1, r)
        c = jnp.where(i >= k, c - width, c)
    return r, c


def _gather_index(t0, width, run=16):
    return _tile_coords(t0, width, (8, LANE), run)[0] * 8 + (_iota((8, LANE), 1) & 7)


def _gather(v, index):
    return jnp.take_along_axis(v, index, axis=1, mode="promise_in_bounds")


def _layernorm(x, eps=1e-5):
    total = lambda a: jnp.sum(jnp.sum(a, axis=1, keepdims=True), axis=0, keepdims=True)
    d = jnp.where(_iota(x.shape, 0) < D // LANE, x - total(x) / D, 0.0)
    return d / jnp.sqrt(total(d * d) / D + eps)


def _mish(u):
    softplus = jnp.log1p(jnp.exp(-jnp.abs(u))) + jnp.where(u > 0, u, 0.0)
    return u * jnp.tanh(softplus)


def _dot(a, b):
    return jnp.dot(a, b, preferred_element_type=F32)


def _loop(lo, hi, body):
    lax.fori_loop(lo, hi, lambda i, carry: (body(i), carry)[1], 0)


def _aligned(i, n):
    return i if isinstance(i, int) else pl.multiple_of(i, n)


def _wait(buf, sem):
    pltpu.make_async_copy(buf, buf, sem).wait()


def _start_in_turns(fence, first, second):
    for i in range(max(len(first), len(second))):
        for queue, copies in enumerate((first, second)):
            if i < len(copies):
                pl.semaphore_signal(fence, 1)
                pl.semaphore_wait(fence, 1)
                copies[i]().start(priority=queue)


def _kernel(x_hbm, k_hbm, v_hbm, wq_hbm, wo_hbm, w1_hbm, b1_hbm, w2_hbm, c_hbm, wm_hbm, o_ref,
            x_v, c_v, b1_v, wm_v, wq_v, wo_v, w1_v, w2_v, kv_v, q_s, p_s, den_s, tab_o, tab_1, tab_2, g_s, acc_s, y_s,
            sem_w, sem_kv, sem_v, sem_w2, fence, *, window):
    _start = functools.partial(_start_in_turns, fence)
    col0 = k_hbm.shape[1] - window
    ncol = window // KV_COLS
    copy = lambda src, dst, sem: functools.partial(pltpu.make_async_copy, src, dst, sem)

    def runs(src, dst, sem, slab, nslab, run):
        at = (pl.ds(slab, nslab), pl.ds(_aligned(run * RUN, RUN), RUN))
        return copy(src.at[at], dst.reshape(src.shape).at[at], sem)

    def mod_a(rs):
        return [runs(wm_hbm, wm_v, sem_w.at[0], s, n, r) for r in rs for s, n in ((0, 4), (4, 3))]

    def mod_b(rs):
        return [runs(*w, sem_w.at[0], s, n, r) for r in rs
                for w, s, n in (((wm_hbm, wm_v), 7, 3), ((w1_hbm, w1_v), 0, 4))]

    def wq(rs):
        return [runs(wq_hbm, wq_v, sem_w.at[1], s, 3, r) for r in rs for s in range(0, 15, 3)]

    def wo(rs):
        return [runs(wo_hbm, wo_v, sem_w.at[1], s, 3, r) for r in rs for s in range(0, 15, 3)]

    def half_head(src, head, slot, which, half, sem_of):
        return [copy(src.at[pl.ds(_aligned(head * DH + r, KV_ROWS), KV_ROWS), pl.ds(col0 + c * KV_COLS, KV_COLS)],
                     kv_v.at[slot, pl.ds(which * DH + r, KV_ROWS), pl.ds(c * KV_COLS, KV_COLS)], sem_of(c))
                for c in range(ncol) for r in range(half * DH // 2, (half + 1) * DH // 2, KV_ROWS)]

    def kv(src, p, which, half):
        slot = (p + (NPAIR if src is v_hbm else 0)) % NSLOT
        return half_head(src, 2 * p + which, slot, which, half, lambda c: sem_kv.at[slot])

    def start_pair(src, p, ahead=None):
        _start(kv(src, p, 0, 0), kv(src, p, 1, 1))
        _start(kv(src, p, 1, 0), ahead or kv(src, p + 1, 0, 1))

    nrun_mod, nrun = wm_hbm.shape[1] // RUN, wq_hbm.shape[1] // RUN
    small = [copy(s, d, sem_w.at[2]) for s, d in ((c_hbm, c_v), (x_hbm, x_v), (b1_hbm, b1_v))]
    _start([], mod_b(range(12)))
    _start(mod_a([0]) + small[:2], mod_b([12]) + small[2:])
    _loop(1, nrun_mod - 12, lambda r: _start(mod_a([r]), mod_b([r + 12])))
    _start(mod_a(range(nrun_mod - 12, nrun_mod)), wo(range(5)))
    start_wq_wo = lambda r: _start(wq([r]), wo([r + 5]))
    for tab, width, run in ((tab_o, 5, 16), (tab_1, F // LANE, 16), (tab_2, 5, 8)):
        for m in range(tab.shape[1]):
            tab[0, m] = _gather_index(run * m, width, run)
            tab[1, m] = _tile_coords(run * m, width, (8, LANE), run)[1] - _iota((8, LANE), 0)
    _loop(0, 10, start_wq_wo)
    for cp in small:
        cp().wait()
    _wait(wm_v, sem_w.at[0])
    _wait(w1_v, sem_w.at[0])

    cf = _rows(c_v[...].astype(F32), D // LANE)
    silu_c = cf * jax.nn.sigmoid(cf)
    width = 6 * D // LANE
    picks = []
    for m in range(width):
        _, col = _tile_coords(16 * m, width, (48, LANE))
        out_row = col
        for i in range(1, 6):
            out_row = jnp.where(col >= 5 * i, out_row + 3, out_row)
        picks.append((_gather(silu_c, _gather_index(16 * m, width)), out_row == _iota((48, LANE), 0)))
    mod = jnp.zeros((48, LANE), F32)
    for j in range(D // LANE):
        lhs = jnp.concatenate([jnp.where(keep, jnp.broadcast_to(g[j:j + 1], (48, LANE)), 0.0).astype(BF16)
                               for g, keep in picks], axis=1)
        mod += _dot(lhs, wm_v[j * width * LANE:(j + 1) * width * LANE, :])
        _loop(10 + 5 * j, 15 + 5 * j, start_wq_wo)
    shift_a, scale_a, gate_a, shift_b, scale_b, gate_b = (mod[8 * i:8 * i + 8] for i in range(6))
    x0 = _rows(x_v[...].astype(F32), D // LANE)
    h = _layernorm(x0) * (1.0 + scale_a) + shift_a
    _loop(35, nrun - 5, start_wq_wo)
    _start(wq(range(nrun - 5, nrun)), kv(k_hbm, 0, 0, 1))

    keep = (_iota((16, LANE), 1) >> 3) == _iota((16, LANE), 0)
    picks = [_gather(h, _gather_index(16 * m, 16)) for m in range(16)]
    lhs = jnp.concatenate([jnp.where(keep, jnp.broadcast_to(g[j:j + 1], (16, LANE)), 0.0).astype(BF16)
                           for j in range(D // LANE) for g in picks], axis=1)
    start_pair(k_hbm, 0)
    _wait(wq_v, sem_w.at[1])
    _wait(wo_v, sem_w.at[1])
    q = []
    for i in range(3):
        q.append(_dot(lhs, wq_v[:, i * LANE:(i + 1) * LANE, :].reshape(-1, LANE)))
        if i < 2:
            _start(kv(k_hbm, 1, i, 0), kv(k_hbm, 1 + i, 1 - i, 1))
    q = jnp.concatenate(q, axis=0)
    row, col = _iota((8, PAIR), 0), _iota((8, PAIR), 1)
    own = jnp.logical_or(jnp.logical_and(row == 0, col < DH), jnp.logical_and(row == 1, col >= DH))
    for p in range(NPAIR):
        qp = jnp.concatenate([jnp.broadcast_to(q[3 * p + u:3 * p + u + 1], (8, LANE)) for u in range(3)], axis=1)
        q_s[p] = jnp.where(own, qp, 0.0)

    def scores(p):
        slot = p % NSLOT
        _wait(kv_v.at[slot], sem_kv.at[slot])
        s = _dot(q_s[p].astype(BF16), kv_v[slot]) * DH ** -0.5
        e = jnp.exp(s - jnp.max(s, axis=-1, keepdims=True))
        p_s[p] = e
        den_s[p] = jnp.broadcast_to(jnp.sum(e, axis=-1, keepdims=True), (8, LANE))

    scores(0)
    _loop(1, NPAIR - 2, lambda p: (start_pair(k_hbm, p + 1), scores(p)))
    start_pair(k_hbm, NPAIR - 1, kv(v_hbm, 0, 0, 1))
    scores(NPAIR - 2)
    start_pair(v_hbm, 0)
    scores(NPAIR - 1)

    def values(p, c0, c1):
        return lax.dot_general(p_s[p, :, c0:c1].astype(BF16), kv_v[(NPAIR + p) % NSLOT, :, c0:c1],
                               (((1,), (1,)), ((), ())), preferred_element_type=F32)

    def spread(v, tab, rows):
        for m in range(tab.shape[1]):
            for r in range(0, v.shape[0], 8):
                g_s[m, r:r + 8] = _gather(v[r:r + 8], tab[0, m])

        def block(i, m, i_high=None):
            g = jnp.broadcast_to(g_s[m, i:i + 1, :], (8, LANE))
            if i_high is not None:
                g = jnp.where(_iota((8, LANE), 1) < LANE // 2, g, jnp.broadcast_to(g_s[m, i_high:i_high + 1, :], (8, LANE)))
            return jnp.concatenate([jnp.where(tab[1, m] == r, g, 0.0) for r in range(0, rows, 8)], axis=0).astype(BF16)

        return block

    def project(p, acc):
        den = den_s[p]
        o = jnp.where(own, acc / jnp.concatenate([den] * 3, axis=1), 0.0)
        block = spread(_rows(jnp.sum(o, axis=0, keepdims=True), 3), tab_o, 8)
        lhs = jnp.concatenate([block(u, m) for u in range(3) for m in range(5)], axis=1)
        return _dot(lhs, wo_v[pl.ds(_aligned(p * 5 * PAIR, 5 * PAIR), 5 * PAIR), :])

    def attend(p, att):
        slot = (NPAIR + p) % NSLOT
        _wait(kv_v.at[slot], sem_kv.at[slot])
        return att + project(p, values(p, 0, window))

    def v_step(p, att):
        start_pair(v_hbm, p + 1)
        return attend(p, att)

    last = NPAIR - 1
    att = lax.fori_loop(0, last - 1, v_step, jnp.zeros((8, LANE), F32))

    slot = (NPAIR + last) % NSLOT
    bounds = [sum(V_LAST[:i]) for i in range(len(V_LAST) + 1)]
    v_sem = lambda c: sem_v.at[sum(c >= b for b in bounds[1:])]
    steps = [sum(W2_STEPS[:i]) for i in range(len(W2_STEPS) + 1)]
    w2 = [copy(w2_hbm.at[pl.ds(2 * (n // 2), 2), pl.ds((n % 2) * 960 + s * 64, 64)], w2_v.at[4 * s + n],
               sem_w2.at[sum(s >= b for b in steps[1:])]) for s in range(steps[-1]) for n in range(4)]
    _start(kv(v_hbm, last, 0, 0), half_head(v_hbm, H - 1, slot, 1, 1, v_sem))
    w2_first, w2_second = w2[0:W2_BOTH:2], w2[1:W2_BOTH:2] + w2[W2_BOTH:]
    _start(half_head(v_hbm, H - 1, slot, 1, 0, v_sem), w2_second[:24])
    att = attend(last - 1, att)
    _start(w2_first, w2_second[24:])
    _wait(kv_v.at[slot, pl.ds(0, DH)], sem_kv.at[slot])
    for i in range(len(V_LAST)):
        c0, c1 = bounds[i] * KV_COLS, bounds[i + 1] * KV_COLS
        _wait(kv_v.at[slot, pl.ds(DH, DH), pl.ds(c0, c1 - c0)], sem_v.at[i])
        acc_s[...] = values(last, c0, c1) + (acc_s[...] if i else 0.0)
    att += project(last, acc_s[...])

    x1 = x0 + gate_a * att
    h2 = _layernorm(x1) * (1.0 + scale_b) + shift_b
    block = spread(h2, tab_1, 16)
    lhs = jnp.concatenate([block(j, m) for j in range(D // LANE) for m in range(F // LANE)], axis=1)
    bias = jnp.concatenate([b1_v[...].astype(F32), jnp.zeros((4, LANE), F32)], axis=0)
    block = spread(_mish(_dot(lhs, w1_v[...]) + bias), tab_2, 8)
    y_s[...] = x1
    for i in range(len(W2_STEPS)):
        lhs = []
        for s in range(steps[i], steps[i + 1]):
            for n in range(4):
                t0 = (n // 2) * 480 + (n % 2) * 120 + s * 8
                lhs.append(block(t0 // 80, t0 % 80 // 8, t0 // 80 + 3))
        blocks = pl.ds(4 * steps[i], 4 * W2_STEPS[i])
        _wait(w2_v.at[blocks], sem_w2.at[i])
        y_s[...] += gate_b * _dot(jnp.concatenate(lhs, axis=1), w2_v[blocks].reshape(-1, LANE))
    out = y_s[...].astype(o_ref.dtype)
    for j in range(D // LANE):
        o_ref[:, j * LANE:(j + 1) * LANE] = out[j:j + 1]


@jax.jit
def pallas_adaLN_cond__sliding_block_cached__dense_activation_mish__decode_kernel(
    A_x: jax.Array,
    A_k_cache: jax.Array,
    A_v_cache: jax.Array,
    A_wq: jax.Array,
    A_wo: jax.Array,
    B_x: jax.Array,
    B_w1: jax.Array,
    B_b1: jax.Array,
    B_w2: jax.Array,
    c: jax.Array,
    w_mod: jax.Array,
):
    del B_x
    sk = A_k_cache.shape[2]
    window = min(4096, max(256, sk // 4))
    kt = jnp.swapaxes(A_k_cache, 2, 3).reshape(H * DH, sk)
    vt = jnp.swapaxes(A_v_cache, 2, 3).reshape(H * DH, sk)
    hbm = pl.BlockSpec(memory_space=pltpu.HBM)
    out = pl.pallas_call(
        functools.partial(_kernel, window=window),
        out_shape=jax.ShapeDtypeStruct((1, D), A_x.dtype),
        in_specs=[hbm] * 10,
        out_specs=pl.BlockSpec(memory_space=pltpu.VMEM),
        scratch_shapes=[
            pltpu.VMEM((1, D), BF16),
            pltpu.VMEM((1, D), BF16),
            pltpu.VMEM((F // LANE, LANE), BF16),
            pltpu.VMEM((D * 6 * D // LANE, LANE), BF16),
            pltpu.VMEM((D // 8, H * DH // 16, LANE), BF16),
            pltpu.VMEM((H * DH * D // LANE, LANE), BF16),
            pltpu.VMEM((D * F // LANE, LANE), BF16),
            pltpu.VMEM((60, 2, 64, LANE), BF16),
            pltpu.VMEM((NSLOT, PAIR, window), BF16),
            pltpu.VMEM((NPAIR, 8, PAIR), F32),
            pltpu.VMEM((NPAIR, 8, window), F32),
            pltpu.VMEM((NPAIR, 8, LANE), F32),
            pltpu.VMEM((2, 5, 8, LANE), jnp.int32),
            pltpu.VMEM((2, 12, 8, LANE), jnp.int32),
            pltpu.VMEM((2, 10, 8, LANE), jnp.int32),
            pltpu.VMEM((12, 16, LANE), F32),
            pltpu.VMEM((8, PAIR), F32),
            pltpu.VMEM((8, LANE), F32),
            pltpu.SemaphoreType.DMA((3,)),
            pltpu.SemaphoreType.DMA((NSLOT,)),
            pltpu.SemaphoreType.DMA((len(V_LAST),)),
            pltpu.SemaphoreType.DMA((len(W2_STEPS),)),
            pltpu.SemaphoreType.REGULAR,
        ],
        compiler_params=pltpu.CompilerParams(
            vmem_limit_bytes=64 * 2**20,
            disable_semaphore_checks=True,
        ),
        name="adaln_attn_mlp_decode",
    )(A_x.reshape(1, D), kt, vt, _tile_major(A_wq, 15), _tile_major(A_wo, 15), _tile_major(B_w1, 4),
      B_b1.reshape(F // LANE, LANE), _tile_major(B_w2, 4), c, _tile_major(w_mod, 10))
    return out.reshape(A_x.shape)
```

```python
import functools

import jax
import jax.numpy as jnp
from jax import lax
import jax.experimental.pallas as pl
import jax.experimental.pallas.tpu as pltpu

D = 640
H = 32
DH = 192
F = 1536
PAIR = 2 * DH
NPAIR = H // 2
LANE = 128
F32 = jnp.float32
BF16 = jnp.bfloat16

SLAB = 2048
RUN = 32
KV_ROWS, KV_COLS = 32, 512
NSLOT = 3
V_LAST = (3, 2, 2, 1)
W2_BOTH = 40
W2_GROUPS = (28, 20, 4, 4, 2, 1, 1)
W2_VPU = 5


def _tile_major(w):
    r, c = w.shape
    return w.reshape(r // 8, 8, c // LANE, LANE).transpose(0, 2, 1, 3).reshape(-1, LANE)


def _iota(shape, dim):
    return lax.broadcasted_iota(jnp.int32, shape, dim)


def _rows(v, n):
    row = _iota((8, LANE), 0)
    out = jnp.zeros((8, LANE), F32)
    for j in range(n):
        out = jnp.where(row == j, jnp.broadcast_to(v[:, j * LANE:(j + 1) * LANE], (8, LANE)), out)
    return out


def _tile_coords(t0, width, shape):
    i = _iota(shape, 1) >> 3
    r = jnp.full(shape, t0 // width, jnp.int32)
    c = i + t0 % width
    for k in range(width - t0 % width, 16, width):
        r = jnp.where(i >= k, r + 1, r)
        c = jnp.where(i >= k, c - width, c)
    return r, c


def _gather_index(t0, width):
    return _tile_coords(t0, width, (8, LANE))[0] * 8 + (_iota((8, LANE), 1) & 7)


def _gather(v, index):
    return jnp.take_along_axis(v, index, axis=1, mode="promise_in_bounds")


def _layernorm(x, eps=1e-5):
    total = lambda a: jnp.sum(jnp.sum(a, axis=1, keepdims=True), axis=0, keepdims=True)
    d = jnp.where(_iota(x.shape, 0) < D // LANE, x - total(x) / D, 0.0)
    return d / jnp.sqrt(total(d * d) / D + eps)


def _mish(u):
    softplus = jnp.log1p(jnp.exp(-jnp.abs(u))) + jnp.where(u > 0, u, 0.0)
    return u * jnp.tanh(softplus)


def _dot(a, b):
    return jnp.dot(a, b, preferred_element_type=F32)


def _loop(lo, hi, body):
    lax.fori_loop(lo, hi, lambda i, carry: (body(i), carry)[1], 0)


def _aligned(i, n):
    return i if isinstance(i, int) else pl.multiple_of(i, n)


def _wait(buf, sem):
    pltpu.make_async_copy(buf, buf, sem).wait()


def _start_in_turns(fence, first, second):
    for i in range(max(len(first), len(second))):
        for queue, copies in enumerate((first, second)):
            if i < len(copies):
                pl.semaphore_signal(fence, 1)
                pl.semaphore_wait(fence, 1)
                copies[i]().start(priority=queue)


def _kernel(x_hbm, k_hbm, v_hbm, wq_hbm, wo_hbm, w1_hbm, b1_hbm, w2_hbm, c_hbm, wm_hbm, o_ref,
            x_v, c_v, b1_v, wm_v, wq_v, wo_v, w1_v, w2_v, kv_v, q_s, p_s, den_s, tab_o, tab_1, g_s, acc_s, y_s, a_s,
            sem_w, sem_kv, sem_v, sem_w2, fence, *, window):
    _start = functools.partial(_start_in_turns, fence)
    col0 = k_hbm.shape[1] - window
    ncol = window // KV_COLS
    copy = lambda src, dst, sem: functools.partial(pltpu.make_async_copy, src, dst, sem)

    def runs(which, slab, nslab, run):
        src, dst, sem = which
        n = src.shape[0] // SLAB
        whole = lambda ref: (ref if ref.shape[0] == n * SLAB else ref.at[pl.ds(0, n * SLAB)]).reshape(n, SLAB, LANE)
        at = (pl.ds(slab, nslab), pl.ds(_aligned(run * RUN, RUN), RUN))
        return copy(whole(src).at[at], whole(dst).at[at], sem)

    def block(which, b):
        src, dst, sem = which
        return copy(src.at[pl.ds(b * LANE, LANE)], dst.at[pl.ds(b * LANE, LANE)], sem)

    wm, w1 = (wm_hbm, wm_v, sem_w.at[0]), (w1_hbm, w1_v, sem_w.at[1])
    wq, wo = (wq_hbm, wq_v.reshape(wq_hbm.shape), sem_w.at[1]), (wo_hbm, wo_v, sem_w.at[1])
    first_a = lambda r: [runs(wm, s, 3, r) for s in (0, 3, 6)]
    first_b = lambda r: [runs(wq, 12, 3, r), runs(wo, 12, 3, r), runs(w1, 0, 3, r)]
    second_a = lambda r: [runs(wq, s, 4, r) for s in (0, 4, 8)]
    second_b = lambda r: [runs(wo, s, 4, r) for s in (0, 4, 8)]
    over = lambda f, rs: [cp for r in rs for cp in f(r)]

    def half_head(src, head, slot, which, half, sem_of):
        return [copy(src.at[pl.ds(_aligned(head * DH + r, KV_ROWS), KV_ROWS), pl.ds(col0 + c * KV_COLS, KV_COLS)],
                     kv_v.at[slot, pl.ds(which * DH + r, KV_ROWS), pl.ds(c * KV_COLS, KV_COLS)], sem_of(c))
                for c in range(ncol) for r in range(half * DH // 2, (half + 1) * DH // 2, KV_ROWS)]

    def kv(src, p, which, half):
        slot = (p + (NPAIR if src is v_hbm else 0)) % NSLOT
        return half_head(src, 2 * p + which, slot, which, half, lambda c: sem_kv.at[slot])

    def start_pair(src, p, ahead=None):
        _start(kv(src, p, 0, 0), kv(src, p, 1, 1))
        _start(kv(src, p, 1, 0), ahead or kv(src, p + 1, 0, 1))

    nrun = SLAB // RUN
    small = [copy(s, d, sem_w.at[2]) for s, d in ((c_hbm, c_v), (x_hbm, x_v), (b1_hbm, b1_v))]
    _start([], [block(w1, 48 + i) for i in (6, 10, 2, 7, 11, 3, 9, 1, 5)] + over(first_b, range(5)))
    _start([block(wm, 144 + i) for i in range(6)] + [block(w1, 48 + i) for i in (0, 4, 8)] + small[:2],
           over(first_b, range(5, 8)) + small[2:])
    for tab, width in ((tab_o, D // LANE), (tab_1, F // LANE)):
        for m in range(width):
            tab[0, m] = _gather_index(16 * m, width)
            tab[1, m] = _tile_coords(16 * m, width, (8, LANE))[1] - _iota((8, LANE), 0)
    _loop(0, nrun - 8, lambda r: _start(first_a(r), first_b(r + 8)))
    _start(over(first_a, range(nrun - 8, nrun)), over(second_b, range(8)))
    start_second = lambda r: _start(second_a(r), second_b(r + 8))
    _loop(0, 16, start_second)
    for cp in small:
        cp().wait()
    _wait(wm_v, sem_w.at[0])

    cf = _rows(c_v[...].astype(F32), D // LANE)
    silu_c = cf * jax.nn.sigmoid(cf)
    width = 6 * D // LANE
    picks = []
    for m in range(width):
        _, col = _tile_coords(16 * m, width, (48, LANE))
        out_row = col
        for i in range(1, 6):
            out_row = jnp.where(col >= 5 * i, out_row + 3, out_row)
        picks.append((_gather(silu_c, _gather_index(16 * m, width)), out_row == _iota((48, LANE), 0)))
    mod = jnp.zeros((48, LANE), F32)
    for j in range(D // LANE):
        lhs = jnp.concatenate([jnp.where(keep, jnp.broadcast_to(g[j:j + 1], (48, LANE)), 0.0).astype(BF16)
                               for g, keep in picks], axis=1)
        mod += _dot(lhs, wm_v[j * width * LANE:(j + 1) * width * LANE, :])
        _loop(16 + 5 * j, 21 + 5 * j, start_second)
    shift_a, scale_a, gate_a, shift_b, scale_b, gate_b = (mod[8 * i:8 * i + 8] for i in range(6))
    x0 = _rows(x_v[...].astype(F32), D // LANE)
    h = _layernorm(x0) * (1.0 + scale_a) + shift_a
    _loop(41, nrun - 8, start_second)
    _start(over(second_a, range(nrun - 8, nrun)), kv(k_hbm, 0, 0, 1))

    keep = (_iota((16, LANE), 1) >> 3) == _iota((16, LANE), 0)
    picks = [_gather(h, _gather_index(16 * m, 16)) for m in range(16)]
    lhs = jnp.concatenate([jnp.where(keep, jnp.broadcast_to(g[j:j + 1], (16, LANE)), 0.0).astype(BF16)
                           for j in range(D // LANE) for g in picks], axis=1)
    start_pair(k_hbm, 0)
    _wait(wq_v, sem_w.at[1])
    _wait(wo_v, sem_w.at[1])
    _wait(w1_v, sem_w.at[1])
    q = []
    for i in range(3):
        q.append(_dot(lhs, wq_v[:, i * LANE:(i + 1) * LANE, :].reshape(-1, LANE)))
        if i < 2:
            _start(kv(k_hbm, 1, i, 0), kv(k_hbm, 1 + i, 1 - i, 1))
    q = jnp.concatenate(q, axis=0)
    row, col = _iota((8, PAIR), 0), _iota((8, PAIR), 1)
    own = jnp.logical_or(jnp.logical_and(row == 0, col < DH), jnp.logical_and(row == 1, col >= DH))
    for p in range(NPAIR):
        qp = jnp.concatenate([jnp.broadcast_to(q[3 * p + u:3 * p + u + 1], (8, LANE)) for u in range(3)], axis=1)
        q_s[p] = jnp.where(own, qp, 0.0)

    def scores(p):
        slot = p % NSLOT
        _wait(kv_v.at[slot], sem_kv.at[slot])
        s = _dot(q_s[p].astype(BF16), kv_v[slot]) * DH ** -0.5
        e = jnp.exp(s - jnp.max(s, axis=-1, keepdims=True))
        p_s[p] = e
        den_s[p] = jnp.broadcast_to(jnp.sum(e, axis=-1, keepdims=True), (8, LANE))

    scores(0)
    _loop(1, NPAIR - 2, lambda p: (start_pair(k_hbm, p + 1), scores(p)))
    start_pair(k_hbm, NPAIR - 1, kv(v_hbm, 0, 0, 1))
    scores(NPAIR - 2)
    start_pair(v_hbm, 0)
    scores(NPAIR - 1)

    def values(p, c0, c1):
        return lax.dot_general(p_s[p, :, c0:c1].astype(BF16), kv_v[(NPAIR + p) % NSLOT, :, c0:c1],
                               (((1,), (1,)), ((), ())), preferred_element_type=F32)

    def spread(v, tab, rows):
        for m in range(tab.shape[1]):
            for r in range(0, v.shape[0], 8):
                g_s[m, r:r + 8] = _gather(v[r:r + 8], tab[0, m])

        def operand(i, m):
            g = jnp.broadcast_to(g_s[m, i:i + 1, :], (8, LANE))
            return jnp.concatenate([jnp.where(tab[1, m] == r, g, 0.0) for r in range(0, rows, 8)], axis=0).astype(BF16)

        return operand

    def project(p, acc):
        den = den_s[p]
        o = jnp.where(own, acc / jnp.concatenate([den] * 3, axis=1), 0.0)
        operand = spread(_rows(jnp.sum(o, axis=0, keepdims=True), 3), tab_o, 8)
        lhs = jnp.concatenate([operand(u, m) for u in range(3) for m in range(5)], axis=1)
        return _dot(lhs, wo_v[pl.ds(_aligned(p * 5 * PAIR, 5 * PAIR), 5 * PAIR), :])

    def attend(p, att):
        slot = (NPAIR + p) % NSLOT
        _wait(kv_v.at[slot], sem_kv.at[slot])
        return att + project(p, values(p, 0, window))

    def v_step(p, att):
        start_pair(v_hbm, p + 1)
        return attend(p, att)

    last = NPAIR - 1
    att = lax.fori_loop(0, last - 1, v_step, jnp.zeros((8, LANE), F32))

    slot = (NPAIR + last) % NSLOT
    bounds = [sum(V_LAST[:i]) for i in range(len(V_LAST) + 1)]
    v_sem = lambda c: sem_v.at[sum(c >= b for b in bounds[1:])]
    order = [15 * n + s for s in range(15) for n in (0, 2, 1, 3)]
    ends = [sum(W2_GROUPS[:i]) for i in range(len(W2_GROUPS) + 1)]
    w2 = [copy(w2_hbm.at[pl.ds(b * LANE, LANE)], w2_v.at[pl.ds(i * LANE, LANE)], sem_w2.at[sum(i >= e for e in ends[1:])])
          for i, b in enumerate(order)]
    _start(kv(v_hbm, last, 0, 0), half_head(v_hbm, H - 1, slot, 1, 1, v_sem))
    w2_first, w2_second = w2[0:W2_BOTH:2], w2[1:W2_BOTH:2] + w2[W2_BOTH:]
    _start(half_head(v_hbm, H - 1, slot, 1, 0, v_sem), w2_second[:24])
    att = attend(last - 1, att)
    _start(w2_first, w2_second[24:])
    _wait(kv_v.at[slot, pl.ds(0, DH)], sem_kv.at[slot])
    for i in range(len(V_LAST)):
        c0, c1 = bounds[i] * KV_COLS, bounds[i + 1] * KV_COLS
        _wait(kv_v.at[slot, pl.ds(DH, DH), pl.ds(c0, c1 - c0)], sem_v.at[i])
        acc_s[...] = values(last, c0, c1) + (acc_s[...] if i else 0.0)
    att += project(last, acc_s[...])

    x1 = x0 + gate_a * att
    h2 = _layernorm(x1) * (1.0 + scale_b) + shift_b
    operand = spread(h2, tab_1, 16)
    lhs = jnp.concatenate([operand(j, m) for j in range(D // LANE) for m in range(F // LANE)], axis=1)
    bias = jnp.concatenate([b1_v[...].astype(F32), jnp.zeros((4, LANE), F32)], axis=0)
    act = _mish(_dot(lhs, w1_v[...]) + bias)
    operand = spread(act, tab_o, 8)
    nmxu = len(W2_GROUPS) - W2_VPU
    first = ends[nmxu]
    row, lane = _iota((8, LANE), 0), _iota((8, LANE), 1)
    for i, b in enumerate(order[first:]):
        column = {}
        for t in range(16 * b, 16 * b + 16):
            r, j = divmod(t, 5)
            if r not in column:
                pick = jnp.where(lane == r % 16 * 8 + row, jnp.broadcast_to(act[r // 16:r // 16 + 1], (8, LANE)), 0.0)
                column[r] = jnp.sum(pick, axis=1, keepdims=True)
            a_s[16 * i + t % 16] = column[r] * gate_b[j:j + 1]
    y_s[...] = x1
    acc = None
    for i in range(len(W2_GROUPS)):
        rows = pl.ds(ends[i] * LANE, W2_GROUPS[i] * LANE)
        _wait(w2_v.at[rows], sem_w2.at[i])
        if i < nmxu:
            lhs = jnp.concatenate([operand(b // 5, b % 5) for b in order[ends[i]:ends[i + 1]]], axis=1)
            y = y_s[...] + gate_b * _dot(lhs, w2_v[rows, :])
            if i < nmxu - 1:
                y_s[...] = y
        else:
            w = w2_v[rows, :].astype(F32)
            acc = acc or [None] * (D // LANE)
            for n in range(16 * W2_GROUPS[i]):
                j = (16 * order[ends[i] + n // 16] + n % 16) % 5
                term = w[8 * n:8 * n + 8] * a_s[16 * (ends[i] - first) + n]
                acc[j] = term if acc[j] is None else acc[j] + term
    for j in range(D // LANE):
        out = jnp.sum(acc[j] + jnp.where(row == j, y, 0.0), axis=0, keepdims=True)
        o_ref[:, j * LANE:(j + 1) * LANE] = out.astype(o_ref.dtype)


@jax.jit
def pallas_adaLN_cond__sliding_block_cached__dense_activation_mish__decode_kernel(
    A_x: jax.Array,
    A_k_cache: jax.Array,
    A_v_cache: jax.Array,
    A_wq: jax.Array,
    A_wo: jax.Array,
    B_x: jax.Array,
    B_w1: jax.Array,
    B_b1: jax.Array,
    B_w2: jax.Array,
    c: jax.Array,
    w_mod: jax.Array,
):
    del B_x
    sk = A_k_cache.shape[2]
    window = min(4096, max(256, sk // 4))
    kt = jnp.swapaxes(A_k_cache, 2, 3).reshape(H * DH, sk)
    vt = jnp.swapaxes(A_v_cache, 2, 3).reshape(H * DH, sk)
    hbm = pl.BlockSpec(memory_space=pltpu.HBM)
    out = pl.pallas_call(
        functools.partial(_kernel, window=window),
        out_shape=jax.ShapeDtypeStruct((1, D), A_x.dtype),
        in_specs=[hbm] * 10,
        out_specs=pl.BlockSpec(memory_space=pltpu.VMEM),
        scratch_shapes=[
            pltpu.VMEM((1, D), BF16),
            pltpu.VMEM((1, D), BF16),
            pltpu.VMEM((F // LANE, LANE), BF16),
            pltpu.VMEM((D * 6 * D // LANE, LANE), BF16),
            pltpu.VMEM((D // 8, H * DH // 16, LANE), BF16),
            pltpu.VMEM((H * DH * D // LANE, LANE), BF16),
            pltpu.VMEM((D * F // LANE, LANE), BF16),
            pltpu.VMEM((F * D // LANE, LANE), BF16),
            pltpu.VMEM((NSLOT, PAIR, window), BF16),
            pltpu.VMEM((NPAIR, 8, PAIR), F32),
            pltpu.VMEM((NPAIR, 8, window), F32),
            pltpu.VMEM((NPAIR, 8, LANE), F32),
            pltpu.VMEM((2, 5, 8, LANE), jnp.int32),
            pltpu.VMEM((2, 12, 8, LANE), jnp.int32),
            pltpu.VMEM((12, 16, LANE), F32),
            pltpu.VMEM((8, PAIR), F32),
            pltpu.VMEM((8, LANE), F32),
            pltpu.VMEM((16 * sum(W2_GROUPS[-W2_VPU:]), 8, LANE), F32),
            pltpu.SemaphoreType.DMA((3,)),
            pltpu.SemaphoreType.DMA((NSLOT,)),
            pltpu.SemaphoreType.DMA((len(V_LAST),)),
            pltpu.SemaphoreType.DMA((len(W2_GROUPS),)),
            pltpu.SemaphoreType.REGULAR,
        ],
        compiler_params=pltpu.CompilerParams(
            vmem_limit_bytes=64 * 2**20,
            disable_semaphore_checks=True,
        ),
        name="adaln_attn_mlp_decode",
    )(A_x.reshape(1, D), kt, vt, _tile_major(A_wq), _tile_major(A_wo), _tile_major(B_w1),
      B_b1.reshape(F // LANE, LANE), _tile_major(B_w2), c, _tile_major(w_mod))
    return out.reshape(A_x.shape)
```

```python
import functools

import jax
import jax.numpy as jnp
from jax import lax
import jax.experimental.pallas as pl
import jax.experimental.pallas.tpu as pltpu

D = 640
H = 32
DH = 192
F = 1536
PAIR = 2 * DH
NPAIR = H // 2
LANE = 128
ND = D // LANE
NF = F // LANE
F32 = jnp.float32
BF16 = jnp.bfloat16

SLAB = 2048
RUN = 32
KV_ROWS, KV_COLS = 32, 512
HALF = 24
LEAD = 25
PITCH = 32
NSLOT = 3
V_GROUPS = (3, 2, 2, 1)
W2_MXU = (28, 16, 8)
W2_VPU = (4, 2, 1, 1)
W2_BOTH = 36


def _tile_major(w):
    r, c = w.shape
    return w.reshape(r // 8, 8, c // LANE, LANE).transpose(0, 2, 1, 3).reshape(-1, LANE)


def _iota(shape, dim):
    return lax.broadcasted_iota(jnp.int32, shape, dim)


def _row(v, i, rows=8):
    return jnp.broadcast_to(v[i:i + 1], (rows, v.shape[1]))


def _stack(v):
    out = jnp.zeros((8, LANE), F32)
    for j in range(v.shape[1] // LANE):
        out = jnp.where(_iota((8, LANE), 0) == j, _row(v[:, j * LANE:(j + 1) * LANE], 0), out)
    return out


def _tile_coords(block, width, shape):
    i = _iota(shape, 1) >> 3
    r0, c0 = divmod(16 * block, width)
    r, c = jnp.full(shape, r0, jnp.int32), i + c0
    for k in range(width - c0, 16, width):
        r = jnp.where(i >= k, r + 1, r)
        c = jnp.where(i >= k, c - width, c)
    return r, c


def _selector(width):
    shape = (LANE, LANE)
    source = lambda m: _tile_coords(m, width, shape)[0] * 8 + (_iota(shape, 1) & 7)
    return jnp.concatenate([jnp.where(source(m) == _iota(shape, 0), 1.0, 0.0).astype(BF16)
                            for m in range(width)], axis=1)


def _layernorm(x, eps=1e-5):
    total = lambda a: jnp.sum(jnp.sum(a, axis=1, keepdims=True), axis=0, keepdims=True)
    d = jnp.where(_iota(x.shape, 0) < ND, x - total(x) / D, 0.0)
    return d / jnp.sqrt(total(d * d) / D + eps)


def _mish(u):
    softplus = jnp.log1p(jnp.exp(-jnp.abs(u))) + jnp.where(u > 0, u, 0.0)
    return u * jnp.tanh(softplus)


def _dot(a, b):
    return jnp.dot(a, b, preferred_element_type=F32)


def _loop(lo, hi, body):
    lax.fori_loop(lo, hi, lambda i, carry: (body(i), carry)[1], 0)


def _aligned(i, n):
    return i if isinstance(i, int) else pl.multiple_of(i, n)


def _shuffled(i):
    return i ^ ((i & 1) << 1)


def _starts(sizes):
    return [sum(sizes[:i]) for i in range(len(sizes) + 1)]


def _wait(buf, sem):
    pltpu.make_async_copy(buf, buf, sem).wait()


def _kernel(x_hbm, k_hbm, v_hbm, wq_hbm, wo_hbm, w1_hbm, b1_hbm, w2_hbm, c_hbm, wm_hbm, o_hbm,
            o_v, x_v, c_v, b1_v, wm_v, wq_v, wo_v, w1_v, w2_v, kv_v,
            q_s, e_s, den_s, sel_d, sel_f, col_d, col_f, g_s, acc_s, y_s, a_s,
            sem_w, sem_kv, sem_v, sem_w2, fence):
    window = kv_v.shape[-1]
    col0 = k_hbm.shape[1] - window
    copy = lambda src, dst, sem: functools.partial(pltpu.make_async_copy, src, dst, sem)

    def start(first, second):
        for i in range(max(len(first), len(second))):
            for queue, copies in enumerate((first, second)):
                if i < len(copies):
                    copies[i]().start(priority=queue)
                    pl.semaphore_signal(fence, 1)
                    pl.semaphore_wait(fence, 1)

    def slot_of(src, p):
        return (p + (NPAIR if src is v_hbm else 0)) % NSLOT

    def half_head(src, p, which, half, sem_of=None):
        slot = slot_of(src, p)
        return [copy(src.at[pl.ds(_aligned(p * PAIR + r, KV_ROWS), KV_ROWS), pl.ds(col0 + c, KV_COLS)],
                     kv_v.at[slot, pl.ds(r, KV_ROWS), pl.ds(c, KV_COLS)],
                     sem_of(c) if sem_of else sem_kv.at[slot])
                for c in (KV_COLS * (i if sem_of else _shuffled(i)) for i in range(window // KV_COLS))
                for r in range(which * DH + (1 - half) * DH // 2, which * DH + (2 - half) * DH // 2, KV_ROWS)]

    def start_head(src, p, which, later=None):
        if later is None:
            later = half_head(src, p + which, 1 - which, 1) + half_head(src, p + 1, which, 1)
        start(half_head(src, p, which, 0), later[LEAD - HALF:LEAD])

    def start_pair(src, p):
        start_head(src, p, 0)
        start_head(src, p, 1)

    def runs(weight, slab, nslab, run):
        src, dst, sem = weight
        at = (pl.ds(slab, nslab), pl.ds(_aligned(run * RUN, RUN), RUN))
        return copy(src.at[at], dst.at[at], sem)

    def blocks(ref, ids):
        per = SLAB // LANE
        return jnp.concatenate([ref[b // per, pl.ds(_aligned(b % per * LANE, LANE), LANE), :] for b in ids], axis=0)

    spots = [(w, b) for first in range(PITCH)
             for w in ((wm_hbm, wm_v, sem_w.at[0]), (w1_hbm, w1_v, sem_w.at[1]))
             for b in range(first, w[0].shape[0] // LANE, PITCH)]
    pieces = lambda spots, n: [copy(src.at[pl.ds(r, n)], dst.at[pl.ds(r, n)], sem)
                               for (src, dst, sem), b in spots for r in range(b * LANE, (b + 1) * LANE, n)]
    small = [copy(s, d, sem_w.at[4 + i]) for i, (s, d) in enumerate(((c_hbm, c_v), (x_hbm, x_v), (b1_hbm, b1_v)))]
    wq, wo = (wq_hbm, wq_v, sem_w.at[2]), (wo_hbm, wo_v, sem_w.at[3])
    first = lambda r: [runs(wq, s, 4, r) for s in (0, 4, 8)]
    second_a = lambda r: [runs(wq, 12, 3, r), runs(wo, 0, 3, r), runs(wo, 3, 3, r)]
    second_b = lambda r: [runs(wo, s, 3, r) for s in (6, 9, 12)]
    over = lambda copies, lo, hi: [cp for r in range(lo, hi) for cp in copies(r)]
    nrun, (lead, skip) = SLAB // RUN, divmod(LEAD, 3)
    other = pieces(spots[1:18:2], LANE) + over(first, 0, nrun) + over(second_b, 0, lead + 1)
    start(pieces(spots[0:16:2], RUN) + small[:2] + pieces(spots[16:17] + spots[18:], LANE),
          other[:32] + small[2:] + other[32:len(other) - 3 + skip])
    start_runs = lambda r: start(second_a(r), (second_b(r + lead) + second_b(r + lead + 1))[skip:skip + 3])
    turn = nrun - lead - 1
    _loop(0, 8, start_runs)
    for sel, col, width in ((sel_d, col_d, ND), (sel_f, col_f, NF)):
        sel[...] = _selector(width)
        for m in range(width):
            col[m] = _tile_coords(m, width, (8, LANE))[1] - _iota((8, LANE), 0)
    _loop(8, 16, start_runs)
    for cp in small:
        cp().wait()
    _wait(wm_v, sem_w.at[0])
    _wait(w1_v, sem_w.at[1])

    c = _stack(c_v[...].astype(F32))
    moved = _dot((c * jax.nn.sigmoid(c)).astype(BF16), _selector(6 * ND))
    keep = []
    for m in range(6 * ND):
        column = out_row = _tile_coords(m, 6 * ND, (48, LANE))[1]
        for i in range(1, 6):
            out_row = jnp.where(column >= ND * i, out_row + 8 - ND, out_row)
        keep.append(out_row == _iota((48, LANE), 0))
    keep = jnp.concatenate(keep, axis=1)
    mod = jnp.zeros((48, LANE), F32)
    for j in range(ND):
        mod += _dot(jnp.where(keep, _row(moved, j, 48), 0.0).astype(BF16), wm_v[j * 6 * D:(j + 1) * 6 * D, :])
        _loop(16 + 6 * j, 22 + 6 * j, start_runs)
    shift_a, scale_a, gate_a, shift_b, scale_b, gate_b = (mod[8 * i:8 * i + 8] for i in range(6))
    x0 = _stack(x_v[...].astype(F32))
    h = _layernorm(x0) * (1.0 + scale_a) + shift_a
    _loop(16 + 6 * ND, turn, start_runs)
    start(over(second_a, turn, nrun),
          second_b(nrun - 1)[skip:] + (half_head(k_hbm, 0, 0, 1) + half_head(k_hbm, 0, 1, 1))[:LEAD])

    moved = _dot(h.astype(BF16), _selector(16))
    keep = ((_iota((16, 16 * LANE), 1) >> 3) & 15) == _iota((16, 16 * LANE), 0)
    lhs = jnp.concatenate([jnp.where(keep, _row(moved, j, 16), 0.0).astype(BF16) for j in range(ND)], axis=1)
    start_pair(k_hbm, 0)
    _wait(wq_v, sem_w.at[2])
    _wait(wo_v, sem_w.at[3])
    q = []
    for i in range(3):
        q.append(_dot(lhs, blocks(wq_v, range(i, 3 * D // 8, 3))))
        if i < 2:
            start_head(k_hbm, 1, i)
    q = jnp.concatenate(q, axis=0)
    row, lane = _iota((8, PAIR), 0), _iota((8, PAIR), 1)
    own = jnp.logical_or(jnp.logical_and(row == 0, lane < DH), jnp.logical_and(row == 1, lane >= DH))
    for p in range(NPAIR):
        q_s[p] = jnp.where(own, jnp.concatenate([_row(q, 3 * p + u) for u in range(3)], axis=1), 0.0)

    def scores(p):
        slot = slot_of(k_hbm, p)
        _wait(kv_v.at[slot], sem_kv.at[slot])
        s = _dot(q_s[p].astype(BF16), kv_v[slot]) * DH ** -0.5
        e = jnp.exp(s - jnp.max(s, axis=-1, keepdims=True))
        e_s[p] = e
        den_s[p] = jnp.broadcast_to(jnp.sum(e, axis=-1, keepdims=True), (8, LANE))

    last = NPAIR - 1
    scores(0)
    _loop(1, last - 1, lambda p: (start_pair(k_hbm, p + 1), scores(p)))
    start_head(k_hbm, last, 0, half_head(k_hbm, last, 1, 1) + half_head(v_hbm, 0, 0, 1))
    start_head(k_hbm, last, 1, half_head(v_hbm, 0, 0, 1) + half_head(v_hbm, 0, 1, 1))
    scores(last - 1)
    start_pair(v_hbm, 0)
    scores(last)

    def values(p, c0, c1):
        return lax.dot_general(e_s[p, :, c0:c1].astype(BF16), kv_v[slot_of(v_hbm, p), :, c0:c1],
                               (((1,), (1,)), ((), ())), preferred_element_type=F32)

    def left_operand(v, sel, col, rows):
        width = col.shape[0]
        g_s[:v.shape[0], :width * LANE] = _dot(v.astype(BF16), sel[...])

        def one(i, m):
            g = _row(g_s[i:i + 1, m * LANE:(m + 1) * LANE], 0)
            return jnp.concatenate([jnp.where(col[m] == r, g, 0.0) for r in range(0, rows, 8)], axis=0)

        return lambda blocks: jnp.concatenate([one(*divmod(b, width)).astype(BF16) for b in blocks], axis=1)

    def project(p, acc):
        o = jnp.where(own, acc / jnp.concatenate([den_s[p]] * 3, axis=1), 0.0)
        lhs = left_operand(_stack(jnp.sum(o, axis=0, keepdims=True)), sel_d, col_d, 8)(range(3 * ND))
        return _dot(lhs, blocks(wo_v, [p * 3 * ND + b for b in range(3 * ND)]))

    def attend(p):
        slot = slot_of(v_hbm, p)
        _wait(kv_v.at[slot], sem_kv.at[slot])
        return project(p, values(p, 0, window))

    def v_step(p, att):
        start_pair(v_hbm, p + 1)
        return att + attend(p)

    att = lax.fori_loop(0, last - 2, v_step, jnp.zeros((8, LANE), F32))

    v_cols = [KV_COLS * n for n in _starts(V_GROUPS)]
    v_sem = lambda c: sem_v.at[sum(c >= e for e in v_cols[1:])]
    order = [ND * NF // 4 * n + s for s in range(ND * NF // 4) for n in (0, 2, 1, 3)]
    w2_at = _starts(W2_MXU + W2_VPU)
    w2 = [copy(w2_hbm.at[pl.ds(b * LANE, LANE)], w2_v.at[pl.ds(i * LANE, LANE)],
               sem_w2.at[sum(i >= e for e in w2_at[1:])]) for i, b in enumerate(order)]
    w2_second = w2[1:W2_BOTH:2] + w2[W2_BOTH:]
    last_half = half_head(v_hbm, last, 1, 1, v_sem)
    start_head(v_hbm, last - 1, 0)
    start_head(v_hbm, last - 1, 1, half_head(v_hbm, last, 0, 1) + last_half)
    att += attend(last - 2)
    start_head(v_hbm, last, 0, last_half + w2_second)
    start(half_head(v_hbm, last, 1, 0, v_sem), w2_second[LEAD - HALF:LEAD])
    att += attend(last - 1)
    start(w2[0:W2_BOTH:2], w2_second[LEAD:])
    slot = slot_of(v_hbm, last)
    _wait(kv_v.at[slot, pl.ds(0, DH)], sem_kv.at[slot])
    for i in range(len(V_GROUPS)):
        _wait(kv_v.at[slot, pl.ds(DH, DH), pl.ds(v_cols[i], v_cols[i + 1] - v_cols[i])], sem_v.at[i])
        acc_s[...] = values(last, v_cols[i], v_cols[i + 1]) + (acc_s[...] if i else 0.0)
    att += project(last, acc_s[...])

    x1 = x0 + gate_a * att
    h = _layernorm(x1) * (1.0 + scale_b) + shift_b
    bias = jnp.concatenate([b1_v[...].astype(F32), jnp.zeros((16 - NF, LANE), F32)], axis=0)
    act = _mish(_dot(left_operand(h, sel_f, col_f, 16)(range(ND * NF)), w1_v[...]) + bias)
    operand = left_operand(act, sel_d, col_d, 8)
    row, lane = _iota((8, LANE), 0), _iota((8, LANE), 1)
    tiles = [16 * b + i for b in order[sum(W2_MXU):] for i in range(16)]
    column = {}
    for n, t in enumerate(tiles):
        r, j = divmod(t, ND)
        if r not in column:
            column[r] = jnp.sum(jnp.where(lane == r % 16 * 8 + row, _row(act, r // 16), 0.0), axis=1, keepdims=True)
        a_s[n] = column[r] * gate_b[j:j + 1]
    y_s[...] = y = x1
    acc = {}
    for i, (b0, b1) in enumerate(zip(w2_at, w2_at[1:])):
        rows = pl.ds(b0 * LANE, (b1 - b0) * LANE)
        _wait(w2_v.at[rows], sem_w2.at[i])
        if i < len(W2_MXU):
            y = y_s[...] + gate_b * _dot(operand(order[b0:b1]), w2_v[rows, :])
            if i < len(W2_MXU) - 1:
                y_s[...] = y
            continue
        w = w2_v[rows, :].astype(F32)
        for n in range(16 * (b1 - b0)):
            m = 16 * (b0 - sum(W2_MXU)) + n
            j = tiles[m] % ND
            term = w[8 * n:8 * n + 8] * a_s[m]
            acc[j] = acc[j] + term if j in acc else term
        if i == len(W2_MXU) + 1:
            acc = {j: acc[j] + jnp.where(row == j, y, 0.0) for j in range(ND)}
    for j in range(ND):
        o_v[:, j * LANE:(j + 1) * LANE] = jnp.sum(acc[j], axis=0, keepdims=True).astype(o_v.dtype)
    out = pltpu.make_async_copy(o_v, o_hbm, sem_w.at[7])
    out.start()
    out.wait()


@jax.jit
def pallas_adaLN_cond__sliding_block_cached__dense_activation_mish__decode_kernel(
    A_x: jax.Array,
    A_k_cache: jax.Array,
    A_v_cache: jax.Array,
    A_wq: jax.Array,
    A_wo: jax.Array,
    B_x: jax.Array,
    B_w1: jax.Array,
    B_b1: jax.Array,
    B_w2: jax.Array,
    c: jax.Array,
    w_mod: jax.Array,
):
    del B_x
    sk = A_k_cache.shape[2]
    window = min(4096, max(256, sk // 4))
    assert window == HALF // 3 * KV_COLS
    kt = jnp.swapaxes(A_k_cache, 2, 3).reshape(H * DH, sk)
    vt = jnp.swapaxes(A_v_cache, 2, 3).reshape(H * DH, sk)
    slabs = (ND * H * DH // SLAB, SLAB, LANE)
    out = pl.pallas_call(
        _kernel,
        out_shape=jax.ShapeDtypeStruct((1, D), A_x.dtype),
        in_specs=[pl.BlockSpec(memory_space=pltpu.HBM)] * 10,
        out_specs=pl.BlockSpec(memory_space=pltpu.HBM),
        scratch_shapes=[
            pltpu.VMEM((1, D), BF16),
            pltpu.VMEM((1, D), BF16),
            pltpu.VMEM((1, D), BF16),
            pltpu.VMEM((NF, LANE), BF16),
            pltpu.VMEM((6 * ND * D, LANE), BF16),
            pltpu.VMEM(slabs, BF16),
            pltpu.VMEM(slabs, BF16),
            pltpu.VMEM((NF * D, LANE), BF16),
            pltpu.VMEM((ND * F, LANE), BF16),
            pltpu.VMEM((NSLOT, PAIR, window), BF16),
            pltpu.VMEM((NPAIR, 8, PAIR), F32),
            pltpu.VMEM((NPAIR, 8, window), F32),
            pltpu.VMEM((NPAIR, 8, LANE), F32),
            pltpu.VMEM((LANE, D), BF16),
            pltpu.VMEM((LANE, F), BF16),
            pltpu.VMEM((ND, 8, LANE), jnp.int32),
            pltpu.VMEM((NF, 8, LANE), jnp.int32),
            pltpu.VMEM((16, F), F32),
            pltpu.VMEM((8, PAIR), F32),
            pltpu.VMEM((8, LANE), F32),
            pltpu.VMEM((16 * sum(W2_VPU), 8, LANE), F32),
            pltpu.SemaphoreType.DMA((8,)),
            pltpu.SemaphoreType.DMA((NSLOT,)),
            pltpu.SemaphoreType.DMA((len(V_GROUPS),)),
            pltpu.SemaphoreType.DMA((len(W2_MXU + W2_VPU),)),
            pltpu.SemaphoreType.REGULAR,
        ],
        compiler_params=pltpu.CompilerParams(
            vmem_limit_bytes=64 * 2**20,
            disable_semaphore_checks=True,
        ),
        name="adaln_attn_mlp_decode",
    )(A_x.reshape(1, D), kt, vt, _tile_major(A_wq).reshape(slabs), _tile_major(A_wo).reshape(slabs),
      _tile_major(B_w1), B_b1.reshape(NF, LANE), _tile_major(B_w2), c, _tile_major(w_mod))
    return out.reshape(A_x.shape)
```
